```python
import jax
import jax.numpy as jnp

def _softmax(x, axis=-1):
    return jax.nn.softmax(x, axis=axis)

def _gelu(x):
    return jax.nn.gelu(x, approximate=True)

def _silu(x):
    return jax.nn.silu(x)

def _sigmoid(x):
    return jax.nn.sigmoid(x)

def _layernorm(x, axis=-1, eps=1e-05):
    m = jnp.mean(x, axis=axis, keepdims=True)
    v = jnp.var(x, axis=axis, keepdims=True)
    return (x - m) / jnp.sqrt(v + eps)

def _scatter_add(tgt, idx, src, axis=0):
    return tgt.at[idx].add(src)

def _segment_sum(src, seg, n):
    return jax.ops.segment_sum(src, seg, n)

class _Rng:

    def __init__(self, key):
        self._k = key

    def _next(self):
        self._k, sub = jax.random.split(self._k)
        return sub

    def normal(self, shape):
        return jax.random.normal(self._next(), shape, dtype=jnp.bfloat16)

    def randint(self, lo, hi, shape):
        return jax.random.randint(self._next(), shape, lo, hi, dtype=jnp.int32)

    def uniform(self, shape, lo=0.0, hi=1.0):
        return jax.random.uniform(self._next(), shape, jnp.bfloat16, lo, hi)

    def permutation(self, n):
        return jax.random.permutation(self._next(), n)
kernel_name = 'interleave_layers__memory_aug_recurrent_mem_tr__ssm_conv_h3__prompt'

def setup_inputs():
    _rng = _Rng(jax.random.key(int.from_bytes(__import__("os").urandom(4), "little")))
    _w = lambda a: (lambda t: t.astype(jnp.bfloat16) if jnp.issubdtype(t.dtype, jnp.floating) else t)(jnp.asarray(a))

    def _A_setup():
        B, S, Dm = (1, 2048, 640)
        H, Dh = (32, 128)
        M, seg = (8, 32)
        seg = min(seg, S)
        S = S // seg * seg
        return {'x': _w((lambda *s: _rng.normal(s) * 0.05)(B, S, Dm)), 'mem0': _w((lambda *s: _rng.normal(s) * 0.05)(B, M, Dm)), 'Wq': _w((lambda *s: _rng.normal(s) * 0.05)(Dm, H, Dh) * Dm ** (-0.5)), 'Wk': _w((lambda *s: _rng.normal(s) * 0.05)(Dm, H, Dh) * Dm ** (-0.5)), 'Wv': _w((lambda *s: _rng.normal(s) * 0.05)(Dm, H, Dh) * Dm ** (-0.5)), 'Wo': _w((lambda *s: _rng.normal(s) * 0.05)(H, Dh, Dm) * (H * Dh) ** (-0.5)), 'seg_len': seg}
    _A_in = _A_setup()

    def _B_setup():
        B, S, D = (1, 2048, 640)
        ks = 4
        return {'q': _w((lambda *s: _rng.normal(s) * 0.05)(B, S, D)), 'k': _w((lambda *s: _rng.normal(s) * 0.05)(B, S, D)), 'v': _w((lambda *s: _rng.normal(s) * 0.05)(B, S, D)), 'shift_k': _w((lambda *s: _rng.normal(s) * 0.05)(D, ks) * 0.5), 'ssm_k': _w((lambda *s: _rng.normal(s) * 0.05)(D, S) * (1.0 / S ** 0.5)), 'ssm_D': _w((lambda *s: _rng.normal(s) * 0.05)(D))}
    _B_in = _B_setup()
    return {'A_x': _A_in['x'], 'A_mem0': _A_in['mem0'], 'A_Wq': _A_in['Wq'], 'A_Wk': _A_in['Wk'], 'A_Wv': _A_in['Wv'], 'A_Wo': _A_in['Wo'], 'A_seg_len': _A_in['seg_len'], 'B_q': _B_in['q'], 'B_k': _B_in['k'], 'B_v': _B_in['v'], 'B_shift_k': _B_in['shift_k'], 'B_ssm_k': _B_in['ssm_k'], 'B_ssm_D': _B_in['ssm_D']}

def reference(A_x, A_mem0, A_Wq, A_Wk, A_Wv, A_Wo, A_seg_len, B_q, B_k, B_v, B_shift_k, B_ssm_k, B_ssm_D):

    def _A_ref(x, mem0, Wq, Wk, Wv, Wo, seg_len):
        B, S, Dm = x.shape
        H, Dh = (Wq.shape[1], Wq.shape[2])
        M = mem0.shape[1]
        scale = Dh ** (-0.5)
        n_seg = S // seg_len
        L = M + seg_len
        idx = jnp.arange(L)
        mask = (idx[:, None] < M) | (idx[:, None] >= idx[None, :])
        mem = mem0
        outs = []
        for s in range(n_seg):
            xs = x[:, s * seg_len:(s + 1) * seg_len, :].copy()
            h = jnp.concatenate([mem, xs], axis=1)
            q = jnp.einsum('btd,dhe->bhte', h, Wq)
            k = jnp.einsum('btd,dhe->bhte', h, Wk)
            v = jnp.einsum('btd,dhe->bhte', h, Wv)
            scores = jnp.einsum('bhqe,bhke->bhqk', q, k) * scale
            scores = jnp.where(mask[None, None], scores, -1000000000.0)
            p = _softmax(scores, axis=-1)
            o = jnp.einsum('bhqk,bhke->bhqe', p, v)
            o = jnp.einsum('bhte,hed->btd', o, Wo)
            mem = o[:, :M, :].copy()
            outs.append(o[:, M:, :])
        return jnp.concatenate(outs, axis=1)

    def _B_ref(q, k, v, shift_k, ssm_k, ssm_D):
        B, S, D = q.shape
        ks = shift_k.shape[-1]
        k_pad = jnp.pad(k, ((0, 0), (ks - 1, 0), (0, 0)))
        k_shift = jnp.zeros_like(k)
        for t in range(ks):
            k_shift = k_shift + k_pad[:, t:t + S, :] * shift_k[:, ks - 1 - t][None, None, :]
        kv = k_shift * v
        L = 2 * S
        kv_pad = jnp.pad(kv, ((0, 0), (0, S), (0, 0)))
        kf_pad = jnp.pad(ssm_k, ((0, 0), (0, S)))
        kv_f = (lambda x, axes=(-2, -1): jnp.fft.rfft2(x.astype(jnp.float32), axes=axes))(kv_pad[:, None, :, :], axes=(1, 2))
        kf_f = (lambda x, axes=(-2, -1): jnp.fft.rfft2(x.astype(jnp.float32), axes=axes))(kf_pad[:, None, :], axes=(1, 2))
        kf_f = (lambda x, *d: x.transpose(*d))(kf_f, 1, 2, 0)
        y_f = kv_f * kf_f[None, :, :, :]
        y = (lambda x, s, axes=(-2, -1): jnp.fft.irfft2(x, s=s, axes=axes).astype(jnp.bfloat16))(y_f, (1, L), axes=(1, 2))[:, 0, :S, :]
        y = y + kv * ssm_D[None, None, :]
        return q * y
    x = A_x
    x = x + _A_ref(_layernorm(x, axis=-1), A_mem0, A_Wq, A_Wk, A_Wv, A_Wo, A_seg_len)
    x = x + _B_ref(_layernorm(x, axis=-1), B_k, B_v, B_shift_k, B_ssm_k, B_ssm_D)
    x = x + _A_ref(_layernorm(x, axis=-1), A_mem0, A_Wq, A_Wk, A_Wv, A_Wo, A_seg_len)
    x = x + _B_ref(_layernorm(x, axis=-1), B_k, B_v, B_shift_k, B_ssm_k, B_ssm_D)
    return x
```

```python
import functools

import numpy as np
import ml_dtypes

import jax
import jax.numpy as jnp
from jax import lax
import jax.experimental.pallas as pl
import jax.experimental.pallas.tpu as pltpu

F32 = jnp.float32
BF16 = jnp.bfloat16
U32 = jnp.uint32

S_LEN = 2048
DM = 640
NH = 32
DH = 128
MEM = 8
SEG = 32
NSEG = S_LEN // SEG
ROWS = 2 * (MEM + SEG)
NSLAB = DM // 128

_NFFT = 2 * S_LEN


def _build_fft_tables():
    n1 = np.zeros(128, np.int64)
    ri = np.zeros(128, np.int64)
    for g in range(8):
        for r in range(2):
            for nl in range(8):
                c = g * 16 + r * 8 + nl
                n1[c] = 8 * g + nl
                ri[c] = r
    fwd = np.zeros((32, 128, 128), np.float64)
    inv = np.zeros((32, 128, 128), np.float64)
    k1 = np.arange(64)
    q_of = n1
    r_of = ri
    for s in range(1, 32):
        ang = -2.0 * np.pi * (n1[None, :] * (s + 64 * k1[:, None])) / _NFFT
        tre, tim = np.cos(ang), np.sin(ang)
        fwd[s, :64] = np.where(ri[None, :] == 0, tre, -tim)
        fwd[s, 64:] = np.where(ri[None, :] == 0, tim, tre)
        nn = np.arange(64)
        ang = 2.0 * np.pi * (nn[:, None] * (s + 64 * q_of[None, :])) / _NFFT
        ure, uim = np.cos(ang) * (2.0 / _NFFT), np.sin(ang) * (2.0 / _NFFT)
        inv[s, :64] = np.where(r_of[None, :] == 0, ure, -uim)
        inv[s, 64:] = np.where(r_of[None, :] == 0, uim, ure)
    f0 = np.zeros((128, 128), np.float64)
    for c in range(128):
        n = n1[c]
        if ri[c] == 0:
            for q in range(32):
                f0[q, c] = np.cos(2 * np.pi * n * q / 64)
                f0[64 + q, c] = (-1.0) ** n if q == 0 else -np.sin(2 * np.pi * n * q / 64)
        else:
            for q in range(32, 64):
                a = -2.0 * np.pi * n * (32 + 64 * (q - 32)) / _NFFT
                f0[q, c] = np.cos(a)
                f0[64 + q, c] = np.sin(a)
    fwd[0] = f0
    g0 = np.zeros((128, 128), np.float64)
    for c in range(128):
        q, r = q_of[c], r_of[c]
        for n in range(64):
            if q < 32:
                if q == 0:
                    g0[n, c] = (1.0 if r == 0 else (-1.0) ** n) / _NFFT
                else:
                    a = 2 * np.pi * n * q / 64
                    g0[n, c] = 2.0 * (np.cos(a) if r == 0 else -np.sin(a)) / _NFFT
            else:
                a = 2.0 * np.pi * n * (32 + 64 * (q - 32)) / _NFFT
                g0[64 + n, c] = 2.0 * (np.cos(a) if r == 0 else -np.sin(a)) / _NFFT
    inv[0] = g0
    return fwd, inv


_FWD64, _INV64 = _build_fft_tables()
_FWD_BF = _FWD64.astype(np.float32).astype(ml_dtypes.bfloat16)
_INV_BF = _INV64.astype(np.float32).astype(ml_dtypes.bfloat16)


class _SV:
    __slots__ = ("x", "s")

    def __init__(self, x, s=1):
        self.x = x
        self.s = s

    def __neg__(self):
        return _SV(self.x, -self.s)

    def __add__(self, o):
        if o is None:
            return self
        if self.s == o.s:
            return _SV(self.x + o.x, self.s)
        if self.s > 0:
            return _SV(self.x - o.x, 1)
        return _SV(o.x - self.x, 1)

    def __sub__(self, o):
        if o is None:
            return self
        return self + (-o)

    def scale(self, c):
        return _SV(self.x * np.float32(c * self.s), 1)

    def get(self):
        return self.x if self.s > 0 else -self.x


def _cfft(re, im, n, sgn):
    if n == 1:
        return re, im
    er, ei = _cfft(re[0::2], im[0::2], n // 2, sgn)
    orr, oi = _cfft(re[1::2], im[1::2], n // 2, sgn)
    outr = [None] * n
    outi = [None] * n
    h = float(np.sqrt(0.5))
    for k in range(n // 2):
        a, b = orr[k], oi[k]
        if k == 0:
            tr, ti = a, b
        elif 4 * k == n:
            tr, ti = (-b, a) if sgn > 0 else (b, -a)
        elif 8 * k == n:
            if sgn < 0:
                tr, ti = (a + b).scale(h), (b - a).scale(h)
            else:
                tr, ti = (a - b).scale(h), (a + b).scale(h)
        elif 8 * k == 3 * n:
            if sgn < 0:
                tr, ti = (b - a).scale(h), (a + b).scale(-h)
            else:
                tr, ti = (a + b).scale(-h), (a - b).scale(h)
        else:
            ang = sgn * 2 * np.pi * k / n
            c, s = float(np.cos(ang)), float(np.sin(ang))
            tr = a.scale(c) - b.scale(s)
            ti = a.scale(s) + b.scale(c)
        outr[k] = er[k] + tr
        outi[k] = ei[k] + ti
        outr[k + n // 2] = er[k] - tr
        outi[k + n // 2] = ei[k] - ti
    return outr, outi


def _odft(u):
    n = len(u)
    if n == 1:
        return [u[0]], [None]
    h = n // 2
    cr, ci = [], []
    for m in range(h):
        a, b = u[m], u[m + h]
        if m == 0:
            cr.append(a)
            ci.append(-b)
        else:
            ang = -2 * np.pi * m / (2 * n)
            c, s = float(np.cos(ang)), float(np.sin(ang))
            if 8 * m == 2 * n:
                hh = float(np.sqrt(0.5))
                cr.append((a - b).scale(hh))
                ci.append((a + b).scale(-hh))
            else:
                cr.append(a.scale(c) + b.scale(s))
                ci.append(a.scale(s) - b.scale(c))
    Cr, Ci = _cfft(cr, ci, h, -1)
    outr = [None] * h
    outi = [None] * h
    for j in range(h):
        if j % 2 == 0:
            outr[j], outi[j] = Cr[j // 2], Ci[j // 2]
        else:
            l = (j - 1) // 2
            outr[j], outi[j] = Cr[h - 1 - l], -Ci[h - 1 - l]
    return outr, outi


def _rdft(x):
    n = len(x)
    if n == 1:
        return [x[0]], [None]
    h = n // 2
    er, ei = _rdft([x[i] + x[i + h] for i in range(h)])
    orr, oi = _odft([x[i] - x[i + h] for i in range(h)])
    outr = [None] * (h + 1)
    outi = [None] * (h + 1)
    for k in range(h + 1):
        if k % 2 == 0:
            outr[k], outi[k] = er[k // 2], ei[k // 2]
        else:
            outr[k], outi[k] = orr[k // 2], oi[k // 2]
    return outr, outi


def _paddft(x):
    n = len(x)
    er, ei = _rdft(x)
    orr, oi = _odft(x)
    outr = [None] * (n + 1)
    outi = [None] * (n + 1)
    for k in range(n + 1):
        if k % 2 == 0:
            outr[k], outi[k] = er[k // 2], ei[k // 2]
        else:
            outr[k], outi[k] = orr[k // 2], oi[k // 2]
    return outr, outi


def _odft_T(sr, si):
    h = len(sr)
    n = 2 * h
    Cr = [None] * h
    Ci = [None] * h
    for j in range(h):
        if j % 2 == 0:
            Cr[j // 2], Ci[j // 2] = sr[j], si[j]
        else:
            l = (j - 1) // 2
            Cr[h - 1 - l], Ci[h - 1 - l] = sr[j], -si[j]
    cr, ci = _cfft(Cr, Ci, h, +1)
    lo, hi = [], []
    for m in range(h):
        if m == 0:
            lo.append(cr[0])
            hi.append(-ci[0])
        else:
            ang = -2 * np.pi * m / (2 * n)
            c, s = float(np.cos(ang)), float(np.sin(ang))
            if 8 * m == 2 * n:
                hh = float(np.sqrt(0.5))
                lo.append((cr[m] - ci[m]).scale(hh))
                hi.append((cr[m] + ci[m]).scale(-hh))
            else:
                lo.append(cr[m].scale(c) + ci[m].scale(s))
                hi.append(cr[m].scale(s) - ci[m].scale(c))
    return lo + hi


def _rdft_T(sr, si):
    h = len(sr) - 1
    if h == 0:
        return [sr[0]]
    ev_r, ev_i = sr[0::2], si[0::2]
    od_r, od_i = sr[1::2], si[1::2]
    s = _rdft_T(ev_r, ev_i)
    if h == 1:
        d = [od_r[0]]
    else:
        d = _odft_T(od_r, od_i)
    return [s[i] + d[i] for i in range(h)] + [s[i] - d[i] for i in range(h)]


def _paddft_T(sr, si):
    n = len(sr) - 1
    a = _rdft_T(sr[0::2], si[0::2])
    b = _odft_T(sr[1::2], si[1::2])
    return [a[i] + b[i] for i in range(n)]


def _mm(a, b):
    return jnp.dot(a, b, preferred_element_type=F32)


def _mm_nt(a, b):
    return lax.dot_general(a, b, (((1,), (1,)), ((), ())), preferred_element_type=F32)


def _ln(x):
    m = jnp.mean(x, axis=-1, keepdims=True)
    d = x - m
    v = jnp.mean(d * d, axis=-1, keepdims=True)
    return d * lax.rsqrt(v + np.float32(1e-5))


def _rb(x):
    return x.astype(BF16).astype(F32)


def _recip(l):
    r = pl.reciprocal(l, approx=True)
    return r * (np.float32(2.0) - l * r)


def _kernel(x_hbm, mem0_hbm, wq_hbm, wk_hbm, wv_hbm, wo_hbm, k_hbm, v_hbm, shift_hbm,
            ssmk_hbm, ssmd_hbm, ffwd_hbm, finv_hbm,
            out_hbm,
            x_v, mem0_v, wbuf, wo_v, k_v, v_v, shift_v, ssmk_v, ssmd_v, ffwd_v, finv_v,
            kf_s, kv_s, akv_s, ah_s, b_s, y_v, out_v, h_s, acc_s, x1p_s, o_s, bias_s,
            sem_b, sem_x, sem_w, sem_wo, sem_out):
    b_cps = []
    for j in range(NSLAB):
        b_cps.append(pltpu.make_async_copy(k_hbm.at[:, pl.ds(j * 128, 128)], k_v.at[j], sem_b.at[0]))
        b_cps.append(pltpu.make_async_copy(v_hbm.at[:, pl.ds(j * 128, 128)], v_v.at[j], sem_b.at[0]))
    b_cps.append(pltpu.make_async_copy(ssmk_hbm, ssmk_v, sem_b.at[0]))
    b_cps.append(pltpu.make_async_copy(shift_hbm, shift_v, sem_b.at[0]))
    b_cps.append(pltpu.make_async_copy(ssmd_hbm, ssmd_v, sem_b.at[0]))
    b_cps.append(pltpu.make_async_copy(ffwd_hbm, ffwd_v, sem_b.at[0]))
    b_cps.append(pltpu.make_async_copy(finv_hbm, finv_v, sem_b.at[0]))
    for c in b_cps:
        c.start()
    x_cps = [pltpu.make_async_copy(x_hbm, x_v, sem_x.at[0]),
             pltpu.make_async_copy(mem0_hbm, mem0_v, sem_x.at[0])]
    for c in x_cps:
        c.start()
    w_cps = []
    for m, w_hbm in enumerate((wq_hbm, wk_hbm, wv_hbm)):
        w32 = w_hbm.bitcast(U32)
        for j in range(32):
            w_cps.append(pltpu.make_async_copy(w32.at[:, j, :], wbuf.at[m * 32 + j], sem_w.at[0]))
    for c in w_cps:
        c.start()
    wo_cp = pltpu.make_async_copy(wo_hbm.bitcast(U32), wo_v, sem_wo.at[0])
    wo_cp.start()

    r_i = lax.broadcasted_iota(jnp.int32, (ROWS, 128), 0)
    c_i = lax.broadcasted_iota(jnp.int32, (ROWS, 128), 1)
    same = jnp.logical_and((r_i < 40) == (c_i < 40), c_i < ROWS)
    memr = jnp.logical_and(r_i >= 32, r_i < 48)
    memc = jnp.logical_and(c_i >= 32, c_i < 48)
    ok = jnp.logical_or(jnp.logical_or(memr, memc), c_i <= r_i)
    log2e = float(np.log2(np.e))
    bias_s[...] = jnp.where(same, jnp.where(ok, np.float32(0.0), np.float32(-1e9 * log2e)),
                            np.float32(-1e30))

    for c in b_cps:
        c.wait()
    kf_s[pl.ds(0, 8), :] = jnp.zeros((8, 128), F32)
    shift_t = shift_v[...]
    row0 = lax.broadcasted_iota(jnp.int32, (8, 128), 0) == 0

    def slab_body(j, carry):
        lane0 = pl.multiple_of(j * 128, 128)
        w = [shift_v[pl.ds(t, 1), pl.ds(lane0, 128)] for t in range(4)]
        dd = ssmd_v[pl.ds(0, 1), pl.ds(lane0, 128)]
        for b in range(S_LEN // 64):
            kf_s[pl.ds(8 + b * 64, 64), :] = k_v[j, pl.ds(b * 64, 64), :].astype(F32)
        for b in range(S_LEN // 64):
            ks = (kf_s[pl.ds(8 + b * 64, 64), :] * w[0] + kf_s[pl.ds(7 + b * 64, 64), :] * w[1]
                  + kf_s[pl.ds(6 + b * 64, 64), :] * w[2] + kf_s[pl.ds(5 + b * 64, 64), :] * w[3])
            kv_s[pl.ds(b * 64, 64), :] = ks * v_v[j, pl.ds(b * 64, 64), :].astype(F32)
        def fwd_stage(dst):
            for g in range(8):
                xs = [_SV(kv_s[pl.ds(n2 * 64 + 8 * g, 8), :]) for n2 in range(32)]
                ar, ai = _paddft(xs)
                for s in range(32):
                    if s == 0:
                        re, im = ar[0].get(), ar[32].get()
                    else:
                        re, im = ar[s].get(), ai[s].get()
                    dst[s, pl.ds(16 * g, 16), :] = jnp.concatenate([re, im], axis=0).astype(BF16)
        fwd_stage(akv_s)
        for b in range(S_LEN // 128):
            blk = ssmk_v[pl.ds(lane0, 128), pl.ds(b * 128, 128)].astype(F32)
            bt = blk.T
            if b == 0:
                top = bt[0:8] + jnp.where(row0, dd, np.float32(0.0))
                kv_s[pl.ds(0, 8), :] = top
                kv_s[pl.ds(8, 120), :] = bt[8:]
            else:
                kv_s[pl.ds(b * 128, 128), :] = bt
        fwd_stage(ah_s)
        for s in range(32):
            f = ffwd_v[s]
            xk = _mm(f, akv_s[s])
            xh = _mm(f, ah_s[s])
            kr, ki, hr, hi = xk[:64], xk[64:], xh[:64], xh[64:]
            yr = kr * hr - ki * hi
            yi = kr * hi + ki * hr
            if s == 0:
                yr0 = jnp.where(row0, kr[:8] * hr[:8], yr[:8])
                yi0 = jnp.where(row0, ki[:8] * hi[:8], yi[:8])
                yr = jnp.concatenate([yr0, yr[8:]], axis=0)
                yi = jnp.concatenate([yi0, yi[8:]], axis=0)
            parts = []
            for jj in range(8):
                parts.append(yr[8 * jj:8 * jj + 8])
                parts.append(yi[8 * jj:8 * jj + 8])
            yb = jnp.concatenate(parts, axis=0).astype(BF16)
            b_s[s] = _mm(finv_v[s], yb)
        for g in range(8):
            sr = [None] * 33
            si = [None] * 33
            sr[0] = _SV(b_s[0, pl.ds(8 * g, 8), :])
            sr[32] = _SV(b_s[0, pl.ds(64 + 8 * g, 8), :])
            for s in range(1, 32):
                sr[s] = _SV(b_s[s, pl.ds(8 * g, 8), :])
                si[s] = _SV(b_s[s, pl.ds(64 + 8 * g, 8), :])
            ys = _paddft_T(sr, si)
            for n2 in range(32):
                y_v[j, pl.ds(n2 * 64 + 8 * g, 8), :] = ys[n2].get()
        return carry

    lax.fori_loop(0, NSLAB, slab_body, 0)

    for c in w_cps:
        c.wait()

    def relayout_body(i, carry):
        m = i // 16
        p = i % 16
        ia = m * 32 + p
        ib = ia + 16
        for r in range(0, 320, 64):
            a = wbuf[ia, pl.ds(r, 64), :]
            b = wbuf[ib, pl.ds(r, 64), :]
            wbuf[ia, pl.ds(r, 64), :] = (a & np.uint32(0xFFFF)) | (b << 16)
            wbuf[ib, pl.ds(r, 64), :] = (a >> 16) | (b & np.uint32(0xFFFF0000))
        return carry

    lax.fori_loop(0, 48, relayout_body, 0)
    wo_cp.wait()
    for c in x_cps:
        c.wait()

    def widx(m, h):
        return m * 32 + (h % 2) * 16 + h // 2

    acc_s[...] = jnp.zeros((ROWS, DM), F32)
    x1p_s[...] = jnp.zeros((SEG, DM), F32)
    cscale = np.float32(DH ** -0.5 * log2e)

    def load_y(idx):
        r0 = pl.multiple_of(idx * SEG, SEG)
        return jnp.concatenate([y_v[jj, pl.ds(r0, SEG), :] for jj in range(NSLAB)], axis=1)

    def l2_epilogue(i):
        a2 = _rb(acc_s[pl.ds(48, 32), :])
        x2 = _rb(x1p_s[...] + a2)
        yy = load_y(jnp.clip(i - 2, 0, NSEG - 1))
        res = x2 + _rb(_rb(_ln(x2)) * yy)
        slot = pl.multiple_of(i * SEG, SEG)
        out_v[pl.ds(slot, SEG), :] = res.astype(BF16)

    def step(i, carry):
        l2_epilogue(i)
        i1 = jnp.clip(i - 1, 0, NSEG - 1)
        r1 = pl.multiple_of(i1 * SEG, SEG)
        a1 = _rb(acc_s[pl.ds(0, 32), :])
        x1 = _rb(x_v[pl.ds(r1, SEG), :].astype(F32) + a1)
        x1p = _rb(x1 + _rb(_rb(_ln(x1)) * load_y(i1)))
        x1p_s[...] = x1p
        h_s[pl.ds(48, 32), :] = _ln(x1p).astype(BF16)
        mem0 = mem0_v[...]
        mems = acc_s[pl.ds(32, 16), :].astype(BF16)
        mem1 = jnp.where(i == 0, mem0, mems[0:8])
        mem2 = jnp.where(i <= 1, mem0, mems[8:16])
        h_s[pl.ds(32, 16), :] = jnp.concatenate([mem1, mem2], axis=0)
        i0 = jnp.minimum(i, NSEG - 1)
        r0 = pl.multiple_of(i0 * SEG, SEG)
        h_s[pl.ds(0, 32), :] = _ln(x_v[pl.ds(r0, SEG), :].astype(F32)).astype(BF16)

        H = h_s[...]
        bias = bias_s[...]
        valid = bias > np.float32(-1.0)
        qkv, P, L = {}, {}, {}

        def wt(m, h):
            return pltpu.bitcast(wbuf[widx(m, h)], BF16)

        def do_qkv(h):
            qkv[h] = tuple(_mm(H, wt(m, h)).astype(BF16) for m in range(3))

        def do_s(h):
            q, k, v = qkv[h]
            kp = jnp.concatenate([k, jnp.zeros((128 - ROWS, DH), BF16)], axis=0)
            sc = _mm_nt(q, kp)
            t = jnp.where(valid, sc * cscale, bias)
            mx = jnp.max(t, axis=-1, keepdims=True)
            e = jnp.exp2(t - mx)
            L[h] = jnp.sum(e, axis=-1, keepdims=True)
            P[h] = e.astype(BF16)

        def do_pv(h):
            v = qkv[h][2]
            vp = jnp.concatenate([v, jnp.zeros((128 - ROWS, DH), BF16)], axis=0)
            o = _mm(P[h], vp) * _recip(L[h])
            o_s[:, pl.ds(h * DH, DH)] = o.astype(BF16)

        for h in range(NH + 3):
            if h < NH:
                do_qkv(h)
            if 2 <= h <= NH + 1:
                do_s(h - 2)
            if 3 <= h:
                do_pv(h - 3)
        for n in range(NSLAB):
            wo_n = pltpu.bitcast(wo_v[:, pl.ds(n * 128, 128)], BF16)
            acc_s[:, pl.ds(n * 128, 128)] = _mm(o_s[...], wo_n)

        @pl.when(i >= 2)
        def _():
            slot = pl.multiple_of(i * SEG, SEG)
            dst = pl.multiple_of((i - 2) * SEG, SEG)
            pltpu.make_async_copy(out_v.at[pl.ds(slot, SEG), :], out_hbm.at[pl.ds(dst, SEG), :],
                                  sem_out.at[0]).start()
        return carry

    lax.fori_loop(0, NSEG + 1, step, 0)
    l2_epilogue(NSEG + 1)
    last = pltpu.make_async_copy(out_v.at[pl.ds((NSEG + 1) * SEG, SEG), :],
                                 out_hbm.at[pl.ds((NSEG - 1) * SEG, SEG), :], sem_out.at[0])
    last.start()
    last.wait()

    def wait_body(i, carry):
        slot = pl.multiple_of(i * SEG, SEG)
        dst = pl.multiple_of((i - 2) * SEG, SEG)
        pltpu.make_async_copy(out_v.at[pl.ds(slot, SEG), :], out_hbm.at[pl.ds(dst, SEG), :],
                              sem_out.at[0]).wait()
        return carry

    lax.fori_loop(2, NSEG + 1, wait_body, 0)


@functools.partial(jax.jit, static_argnames=("A_seg_len",))
def pallas_interleave_layers__memory_aug_recurrent_mem_tr__ssm_conv_h3__prompt_kernel(
    A_x, A_mem0, A_Wq, A_Wk, A_Wv, A_Wo, A_seg_len, B_q, B_k, B_v, B_shift_k, B_ssm_k, B_ssm_D,
):
    del B_q
    assert A_seg_len == SEG
    x = A_x.reshape(S_LEN, DM)
    mem0 = A_mem0.reshape(MEM, DM)
    wq = A_Wq.reshape(DM // 2, 2 * NH, DH)
    wk = A_Wk.reshape(DM // 2, 2 * NH, DH)
    wv = A_Wv.reshape(DM // 2, 2 * NH, DH)
    wo = A_Wo.reshape(NH * DH, DM)
    k = B_k.reshape(S_LEN, DM)
    v = B_v.reshape(S_LEN, DM)
    shift = jnp.pad(B_shift_k.T.astype(F32), ((0, 4), (0, 0)))
    ssmd = jnp.pad(B_ssm_D.reshape(1, DM).astype(F32), ((0, 7), (0, 0)))
    ffwd = jnp.asarray(_FWD_BF)
    finv = jnp.asarray(_INV_BF)
    any_spec = pl.BlockSpec(memory_space=pl.ANY)
    V = pltpu.VMEM
    scratch = [
        V((S_LEN, DM), BF16),
        V((MEM, DM), BF16),
        V((96, DM // 2, DH), U32),
        V((NH * DH // 2, DM), U32),
        V((NSLAB, S_LEN, 128), BF16),
        V((NSLAB, S_LEN, 128), BF16),
        V((8, DM), F32),
        V((DM, S_LEN), BF16),
        V((8, DM), F32),
        V((32, 128, 128), BF16),
        V((32, 128, 128), BF16),
        V((8 + S_LEN, 128), F32),
        V((S_LEN, 128), F32),
        V((32, 128, 128), BF16),
        V((32, 128, 128), BF16),
        V((32, 128, 128), F32),
        V((NSLAB, S_LEN, 128), F32),
        V(((NSEG + 2) * SEG, DM), BF16),
        V((ROWS, DM), BF16),
        V((ROWS, DM), F32),
        V((SEG, DM), F32),
        V((ROWS, NH * DH), BF16),
        V((ROWS, 128), F32),
        pltpu.SemaphoreType.DMA((1,)),
        pltpu.SemaphoreType.DMA((1,)),
        pltpu.SemaphoreType.DMA((1,)),
        pltpu.SemaphoreType.DMA((1,)),
        pltpu.SemaphoreType.DMA((1,)),
    ]
    out = pl.pallas_call(
        _kernel,
        out_shape=jax.ShapeDtypeStruct((S_LEN, DM), BF16),
        in_specs=[any_spec] * 13,
        out_specs=any_spec,
        scratch_shapes=scratch,
        compiler_params=pltpu.CompilerParams(vmem_limit_bytes=100 * 1024 * 1024),
    )(x, mem0, wq, wk, wv, wo, k, v, shift, B_ssm_k, ssmd, ffwd, finv)
    return out.reshape(1, S_LEN, DM)
```

```python
import functools

import numpy as np
import ml_dtypes

import jax
import jax.numpy as jnp
from jax import lax
import jax.experimental.pallas as pl
import jax.experimental.pallas.tpu as pltpu

F32 = jnp.float32
BF16 = jnp.bfloat16
U32 = jnp.uint32

S_LEN = 2048
DM = 640
NH = 32
DH = 128
MEM = 8
SEG = 32
NSEG = S_LEN // SEG
ROWS = 2 * (MEM + SEG)
NSLAB = DM // 128

_NFFT = 2 * S_LEN


def _build_fft_tables():
    n1 = np.zeros(128, np.int64)
    ri = np.zeros(128, np.int64)
    for g in range(8):
        for r in range(2):
            for nl in range(8):
                c = g * 16 + r * 8 + nl
                n1[c] = 8 * g + nl
                ri[c] = r
    fwd = np.zeros((32, 128, 128), np.float64)
    inv = np.zeros((32, 128, 128), np.float64)
    k1 = np.arange(64)
    q_of = n1
    r_of = ri
    for s in range(1, 32):
        ang = -2.0 * np.pi * (n1[None, :] * (s + 64 * k1[:, None])) / _NFFT
        tre, tim = np.cos(ang), np.sin(ang)
        fwd[s, :64] = np.where(ri[None, :] == 0, tre, -tim)
        fwd[s, 64:] = np.where(ri[None, :] == 0, tim, tre)
        nn = np.arange(64)
        ang = 2.0 * np.pi * (nn[:, None] * (s + 64 * q_of[None, :])) / _NFFT
        ure, uim = np.cos(ang) * (2.0 / _NFFT), np.sin(ang) * (2.0 / _NFFT)
        inv[s, :64] = np.where(r_of[None, :] == 0, ure, -uim)
        inv[s, 64:] = np.where(r_of[None, :] == 0, uim, ure)
    f0 = np.zeros((128, 128), np.float64)
    for c in range(128):
        n = n1[c]
        if ri[c] == 0:
            for q in range(32):
                f0[q, c] = np.cos(2 * np.pi * n * q / 64)
                f0[64 + q, c] = (-1.0) ** n if q == 0 else -np.sin(2 * np.pi * n * q / 64)
        else:
            for q in range(32, 64):
                a = -2.0 * np.pi * n * (32 + 64 * (q - 32)) / _NFFT
                f0[q, c] = np.cos(a)
                f0[64 + q, c] = np.sin(a)
    fwd[0] = f0
    g0 = np.zeros((128, 128), np.float64)
    for c in range(128):
        q, r = q_of[c], r_of[c]
        for n in range(64):
            if q < 32:
                if q == 0:
                    g0[n, c] = (1.0 if r == 0 else (-1.0) ** n) / _NFFT
                else:
                    a = 2 * np.pi * n * q / 64
                    g0[n, c] = 2.0 * (np.cos(a) if r == 0 else -np.sin(a)) / _NFFT
            else:
                a = 2.0 * np.pi * n * (32 + 64 * (q - 32)) / _NFFT
                g0[64 + n, c] = 2.0 * (np.cos(a) if r == 0 else -np.sin(a)) / _NFFT
    inv[0] = g0
    return fwd, inv


_FWD64, _INV64 = _build_fft_tables()
_FWD_BF = _FWD64.astype(np.float32).astype(ml_dtypes.bfloat16)
_INV_BF = _INV64.astype(np.float32).astype(ml_dtypes.bfloat16)


class _SV:
    __slots__ = ("x", "s")

    def __init__(self, x, s=1):
        self.x = x
        self.s = s

    def __neg__(self):
        return _SV(self.x, -self.s)

    def __add__(self, o):
        if o is None:
            return self
        if self.s == o.s:
            return _SV(self.x + o.x, self.s)
        if self.s > 0:
            return _SV(self.x - o.x, 1)
        return _SV(o.x - self.x, 1)

    def __sub__(self, o):
        if o is None:
            return self
        return self + (-o)

    def scale(self, c):
        return _SV(self.x * np.float32(c * self.s), 1)

    def get(self):
        return self.x if self.s > 0 else -self.x


def _cfft(re, im, n, sgn):
    if n == 1:
        return re, im
    er, ei = _cfft(re[0::2], im[0::2], n // 2, sgn)
    orr, oi = _cfft(re[1::2], im[1::2], n // 2, sgn)
    outr = [None] * n
    outi = [None] * n
    h = float(np.sqrt(0.5))
    for k in range(n // 2):
        a, b = orr[k], oi[k]
        if k == 0:
            tr, ti = a, b
        elif 4 * k == n:
            tr, ti = (-b, a) if sgn > 0 else (b, -a)
        elif 8 * k == n:
            if sgn < 0:
                tr, ti = (a + b).scale(h), (b - a).scale(h)
            else:
                tr, ti = (a - b).scale(h), (a + b).scale(h)
        elif 8 * k == 3 * n:
            if sgn < 0:
                tr, ti = (b - a).scale(h), (a + b).scale(-h)
            else:
                tr, ti = (a + b).scale(-h), (a - b).scale(h)
        else:
            ang = sgn * 2 * np.pi * k / n
            c, s = float(np.cos(ang)), float(np.sin(ang))
            tr = a.scale(c) - b.scale(s)
            ti = a.scale(s) + b.scale(c)
        outr[k] = er[k] + tr
        outi[k] = ei[k] + ti
        outr[k + n // 2] = er[k] - tr
        outi[k + n // 2] = ei[k] - ti
    return outr, outi


def _odft(u):
    n = len(u)
    if n == 1:
        return [u[0]], [None]
    h = n // 2
    cr, ci = [], []
    for m in range(h):
        a, b = u[m], u[m + h]
        if m == 0:
            cr.append(a)
            ci.append(-b)
        else:
            ang = -2 * np.pi * m / (2 * n)
            c, s = float(np.cos(ang)), float(np.sin(ang))
            if 8 * m == 2 * n:
                hh = float(np.sqrt(0.5))
                cr.append((a - b).scale(hh))
                ci.append((a + b).scale(-hh))
            else:
                cr.append(a.scale(c) + b.scale(s))
                ci.append(a.scale(s) - b.scale(c))
    Cr, Ci = _cfft(cr, ci, h, -1)
    outr = [None] * h
    outi = [None] * h
    for j in range(h):
        if j % 2 == 0:
            outr[j], outi[j] = Cr[j // 2], Ci[j // 2]
        else:
            l = (j - 1) // 2
            outr[j], outi[j] = Cr[h - 1 - l], -Ci[h - 1 - l]
    return outr, outi


def _rdft(x):
    n = len(x)
    if n == 1:
        return [x[0]], [None]
    h = n // 2
    er, ei = _rdft([x[i] + x[i + h] for i in range(h)])
    orr, oi = _odft([x[i] - x[i + h] for i in range(h)])
    outr = [None] * (h + 1)
    outi = [None] * (h + 1)
    for k in range(h + 1):
        if k % 2 == 0:
            outr[k], outi[k] = er[k // 2], ei[k // 2]
        else:
            outr[k], outi[k] = orr[k // 2], oi[k // 2]
    return outr, outi


def _paddft(x):
    n = len(x)
    er, ei = _rdft(x)
    orr, oi = _odft(x)
    outr = [None] * (n + 1)
    outi = [None] * (n + 1)
    for k in range(n + 1):
        if k % 2 == 0:
            outr[k], outi[k] = er[k // 2], ei[k // 2]
        else:
            outr[k], outi[k] = orr[k // 2], oi[k // 2]
    return outr, outi


def _odft_T(sr, si):
    h = len(sr)
    n = 2 * h
    Cr = [None] * h
    Ci = [None] * h
    for j in range(h):
        if j % 2 == 0:
            Cr[j // 2], Ci[j // 2] = sr[j], si[j]
        else:
            l = (j - 1) // 2
            Cr[h - 1 - l], Ci[h - 1 - l] = sr[j], -si[j]
    cr, ci = _cfft(Cr, Ci, h, +1)
    lo, hi = [], []
    for m in range(h):
        if m == 0:
            lo.append(cr[0])
            hi.append(-ci[0])
        else:
            ang = -2 * np.pi * m / (2 * n)
            c, s = float(np.cos(ang)), float(np.sin(ang))
            if 8 * m == 2 * n:
                hh = float(np.sqrt(0.5))
                lo.append((cr[m] - ci[m]).scale(hh))
                hi.append((cr[m] + ci[m]).scale(-hh))
            else:
                lo.append(cr[m].scale(c) + ci[m].scale(s))
                hi.append(cr[m].scale(s) - ci[m].scale(c))
    return lo + hi


def _rdft_T(sr, si):
    h = len(sr) - 1
    if h == 0:
        return [sr[0]]
    ev_r, ev_i = sr[0::2], si[0::2]
    od_r, od_i = sr[1::2], si[1::2]
    s = _rdft_T(ev_r, ev_i)
    if h == 1:
        d = [od_r[0]]
    else:
        d = _odft_T(od_r, od_i)
    return [s[i] + d[i] for i in range(h)] + [s[i] - d[i] for i in range(h)]


def _paddft_T(sr, si):
    n = len(sr) - 1
    a = _rdft_T(sr[0::2], si[0::2])
    b = _odft_T(sr[1::2], si[1::2])
    return [a[i] + b[i] for i in range(n)]


def _mm(a, b):
    return jnp.dot(a, b, preferred_element_type=F32)


def _mm_nt(a, b):
    return lax.dot_general(a, b, (((1,), (1,)), ((), ())), preferred_element_type=F32)


def _ln(x):
    m = jnp.mean(x, axis=-1, keepdims=True)
    d = x - m
    v = jnp.mean(d * d, axis=-1, keepdims=True)
    return d * lax.rsqrt(v + np.float32(1e-5))


def _rb(x):
    return x.astype(BF16).astype(F32)


def _recip(l):
    r = pl.reciprocal(l, approx=True)
    return r * (np.float32(2.0) - l * r)


def _pack_rows_u32(t):
    u = t.view(np.uint16).astype(np.uint32)
    return u[:, 0::2, :] | (u[:, 1::2, :] << 16)


_FTAB_U32 = _pack_rows_u32(np.concatenate([_FWD_BF, _INV_BF], axis=0))


def _kernel(x_hbm, mem0_hbm, wq_hbm, wk_hbm, wv_hbm, wo_hbm, k_hbm, v_hbm, shift_hbm,
            ssmk_hbm, ssmd_hbm, ftab_hbm,
            out_hbm,
            x_v, mem0_v, wbuf, wo_v, k_v, v_v, shift_v, ssmk_v, ssmd_v, ftab_v, wrow_s,
            kf_s, kv_s, ht_s, akv_s, ah_s, ba_s, bb_s, ta_s, y_v, out_v, h_s, q1_s, x1p_s, bias_s, biasl_s,
            sem_f, sem_s, sem_x, sem_w, sem_wo, sem_out):
    def slab_copies(j):
        return [pltpu.make_async_copy(k_hbm.at[:, pl.ds(j * 128, 128)], k_v.at[j], sem_s.at[j]),
                pltpu.make_async_copy(v_hbm.at[:, pl.ds(j * 128, 128)], v_v.at[j], sem_s.at[j]),
                pltpu.make_async_copy(ssmk_hbm.at[pl.ds(j * 128, 128), :], ssmk_v.at[j], sem_s.at[j])]

    f_cps = [pltpu.make_async_copy(shift_hbm, shift_v, sem_f.at[0]),
             pltpu.make_async_copy(ssmd_hbm, ssmd_v, sem_f.at[0]),
             pltpu.make_async_copy(ftab_hbm, ftab_v, sem_f.at[0])]
    XA = 4 * SEG
    xa_cps = [pltpu.make_async_copy(x_hbm.at[pl.ds(0, XA), :], x_v.at[pl.ds(0, XA), :], sem_x.at[0]),
              pltpu.make_async_copy(mem0_hbm, mem0_v, sem_x.at[0])]
    xb_cp = pltpu.make_async_copy(x_hbm.at[pl.ds(XA, S_LEN - XA), :], x_v.at[pl.ds(XA, S_LEN - XA), :],
                                  sem_x.at[1])
    w_cps = []
    for m, w_hbm in enumerate((wq_hbm, wk_hbm, wv_hbm)):
        w32 = w_hbm.bitcast(U32)
        for j in range(32):
            w_cps.append(pltpu.make_async_copy(w32.at[:, j, :], wbuf.at[m * 32 + j], sem_w.at[0]))
    wo_cp = pltpu.make_async_copy(wo_hbm.bitcast(U32), wo_v, sem_wo.at[0])

    for c in f_cps + slab_copies(0):
        c.start()

    r_i = lax.broadcasted_iota(jnp.int32, (ROWS, 128), 0)
    c_i = lax.broadcasted_iota(jnp.int32, (ROWS, 128), 1)
    same = jnp.logical_and((r_i < 40) == (c_i < 40), c_i < ROWS)
    memr = jnp.logical_and(r_i >= 32, r_i < 48)
    memc = jnp.logical_and(c_i >= 32, c_i < 48)
    ok = jnp.logical_or(jnp.logical_or(memr, memc), c_i <= r_i)
    log2e = float(np.log2(np.e))
    bias_s[...] = jnp.where(same, jnp.where(ok, np.float32(0.0), np.float32(-1e9 * log2e)),
                            np.float32(-1e30))
    r_l = lax.broadcasted_iota(jnp.int32, (48, 128), 0) + 32
    c_l = lax.broadcasted_iota(jnp.int32, (48, 128), 1) + 32
    same_l = jnp.logical_and((r_l < 40) == (c_l < 40), c_l < ROWS)
    ok_l = jnp.logical_or(jnp.logical_or(r_l < 48, c_l < 48), c_l <= r_l)
    biasl_s[...] = jnp.where(same_l, jnp.where(ok_l, np.float32(0.0), np.float32(-1e9 * log2e)),
                             np.float32(-1e30))
    kf_s[pl.ds(0, 8), :] = jnp.zeros((8, 128), F32)

    def zero_b(i, c):
        bb_s[i] = jnp.zeros((128, 128), F32)
        return c


    for c in f_cps + slab_copies(0):
        c.wait()
    for c in slab_copies(1) + slab_copies(2):
        c.start()
    wrow_s[pl.ds(0, 4), :] = shift_v[...].astype(F32).T
    wrow_s[pl.ds(4, 1), :] = ssmd_v[...].astype(F32).reshape(1, DM)
    row0 = lax.broadcasted_iota(jnp.int32, (8, 128), 0) == 0
    RB = 128

    def taps(j):
        lane0 = j * 128
        return ([wrow_s[pl.ds(t, 1), pl.ds(lane0, 128)] for t in range(4)],
                wrow_s[pl.ds(4, 1), pl.ds(lane0, 128)])

    def prep_p(j, r, n):
        kf_s[pl.ds(8 + r, n), :] = k_v[j, pl.ds(r, n), :].astype(F32)

    def prep_q(j, r, w):
        ks = (kf_s[pl.ds(8 + r, RB), :] * w[0] + kf_s[pl.ds(7 + r, RB), :] * w[1]
              + kf_s[pl.ds(6 + r, RB), :] * w[2] + kf_s[pl.ds(5 + r, RB), :] * w[3])
        kv_s[pl.ds(r, RB), :] = ks * v_v[j, pl.ds(r, RB), :].astype(F32)

    def prep_t(j, dd):
        ht = ssmk_v[j].astype(F32).T
        ht_s[pl.ds(8, S_LEN - 8), :] = ht[8:]
        ht_s[pl.ds(0, 8), :] = ht[:8] + jnp.where(row0, dd, np.float32(0.0))

    def pk(re, im):
        return jnp.concatenate([re, im], axis=0).astype(BF16)

    def fwd_nets(src, dst):
        def fwd_a(g, c):
            r = pl.multiple_of(g * 8, 8)
            r2 = pl.multiple_of(g * 16, 16)
            xs = [_SV(src[pl.ds(n2 * 64 + r, 8), :]) for n2 in range(32)]
            orr, oi = _odft(xs)
            for q in range(16):
                dst[2 * q + 1, pl.ds(r2, 16), :] = pk(orr[q].get(), oi[q].get())
            return c

        def fwd_b(g, c):
            r = pl.multiple_of(g * 8, 8)
            r2 = pl.multiple_of(g * 16, 16)
            xs = [_SV(src[pl.ds(n2 * 64 + r, 8), :]) for n2 in range(32)]
            er, ei = _rdft(xs)
            dst[0, pl.ds(r2, 16), :] = pk(er[0].get(), er[16].get())
            for q in range(1, 16):
                dst[2 * q, pl.ds(r2, 16), :] = pk(er[q].get(), ei[q].get())
            return c

        lax.fori_loop(0, 8, fwd_a, 0)
        lax.fori_loop(0, 8, fwd_b, 0)

    def inv_a(br, r):
        sr = [_SV(br[2 * q + 1, pl.ds(r, 8), :]) for q in range(16)]
        si = [_SV(br[2 * q + 1, pl.ds(64 + r, 8), :]) for q in range(16)]
        bb = _odft_T(sr, si)
        for n2 in range(32):
            ta_s[pl.ds(n2 * 64 + r, 8), :] = bb[n2].get()

    def inv_b(br, jy, r):
        sr = [None] * 17
        si = [None] * 17
        sr[0] = _SV(br[0, pl.ds(r, 8), :])
        sr[16] = _SV(br[0, pl.ds(64 + r, 8), :])
        for q in range(1, 16):
            sr[q] = _SV(br[2 * q, pl.ds(r, 8), :])
            si[q] = _SV(br[2 * q, pl.ds(64 + r, 8), :])
        aa = _rdft_T(sr, si)
        for n2 in range(32):
            prev = _SV(ta_s[pl.ds(n2 * 64 + r, 8), :])
            y_v[jy, pl.ds(n2 * 64 + r, 8), :] = (aa[n2] + prev).get()

    def mxu_block(j, bw, br):
        jn = j + 1
        jy = j - 1
        do_prep = j + 1 < NSL
        do_inv = j >= 1
        w, dd = taps(min(jn, NSLAB - 1))
        LAG = 3
        X, Y = {}, {}
        for t in range(32 + LAG):
            if do_prep and t % 8 == 0 and t < 32:
                nb = t // 2
                ht_s[pl.ds(nb * 128, 512), :] = ssmk_v[jn, :, pl.ds(nb * 128, 512)].astype(F32).T
            if do_prep and t % 2 == 0 and t < 32:
                prep_p(jn, (t // 2) * RB, RB)
            if do_prep and t % 2 == 1 and t < 32:
                prep_q(jn, (t // 2) * RB, w)
            if do_inv and t % 4 == 0 and t < 32:
                inv_a(br, (t // 4) * 8)
            if do_inv and t % 4 == 2 and t < 32:
                inv_b(br, jy, (t // 4) * 8)
            if t < 32:
                f = pltpu.bitcast(ftab_v[t], BF16)
                X[t] = (_mm(f, akv_s[t]), _mm(f, ah_s[t]))
            if 1 <= t <= 32:
                sl = t - 1
                xk, xh = X.pop(sl)
                kr, ki, hr, hi = xk[:64], xk[64:], xh[:64], xh[64:]
                yr = kr * hr - ki * hi
                yi = kr * hi + ki * hr
                if sl == 0:
                    yr = jnp.concatenate([jnp.where(row0, kr[:8] * hr[:8], yr[:8]), yr[8:]], axis=0)
                    yi = jnp.concatenate([jnp.where(row0, ki[:8] * hi[:8], yi[:8]), yi[8:]], axis=0)
                parts = []
                for jj in range(8):
                    parts.append(yr[8 * jj:8 * jj + 8])
                    parts.append(yi[8 * jj:8 * jj + 8])
                Y[sl] = jnp.concatenate(parts, axis=0).astype(BF16)
            if t >= LAG:
                sl = t - LAG
                bw[sl] = _mm(pltpu.bitcast(ftab_v[32 + sl], BF16), Y.pop(sl))
        if do_prep:
            ht_s[pl.ds(0, 8), :] = ht_s[pl.ds(0, 8), :] + jnp.where(row0, dd, np.float32(0.0))

    NSL = NSLAB
    w0, dd0 = taps(0)

    def p_body(b, c):
        prep_p(0, pl.multiple_of(b * 256, 256), 256)
        return c

    lax.fori_loop(0, S_LEN // 256, p_body, 0)

    def q_body(b, c):
        prep_q(0, pl.multiple_of(b * RB, RB), w0)
        return c

    lax.fori_loop(0, S_LEN // RB, q_body, 0)
    prep_t(0, dd0)

    NSL = NSLAB

    for j in range(NSL):
        fwd_nets(kv_s, akv_s)
        fwd_nets(ht_s, ah_s)
        if j == 0:
            for c in slab_copies(1) + slab_copies(2):
                c.wait()
            for c in slab_copies(3) + slab_copies(4) + xa_cps:
                c.start()
        if j == 1:
            for c in slab_copies(3) + slab_copies(4) + xa_cps:
                c.wait()
            for c in w_cps:
                c.start()
        mxu_block(j, (ba_s, bb_s)[j % 2], (ba_s, bb_s)[1 - j % 2])
    jl = NSL - 1

    def ia_body(g, c):
        inv_a(ba_s if jl % 2 == 0 else bb_s, pl.multiple_of(g * 8, 8))
        return c

    def ib_body(g, c):
        inv_b(ba_s if jl % 2 == 0 else bb_s, jl, pl.multiple_of(g * 8, 8))
        return c

    lax.fori_loop(0, 8, ia_body, 0)
    lax.fori_loop(0, 8, ib_body, 0)

    for c in w_cps:
        c.wait()
    wo_cp.start()

    def relayout_body(i, carry):
        m = i // 16
        p = i % 16
        ia = m * 32 + p
        ib = ia + 16
        for r in range(0, 320, 64):
            a = wbuf[ia, pl.ds(r, 64), :]
            b = wbuf[ib, pl.ds(r, 64), :]
            wbuf[ia, pl.ds(r, 64), :] = (a & np.uint32(0xFFFF)) | (b << 16)
            wbuf[ib, pl.ds(r, 64), :] = (a >> 16) | (b & np.uint32(0xFFFF0000))
        return carry

    lax.fori_loop(0, 48, relayout_body, 0)

    def widx(m, h):
        return m * 32 + (h % 2) * 16 + h // 2

    NF = 3
    G = 8
    LAG_S = 2
    LAG_PV = 3
    LAG_WO = 4
    cscale = np.float32(DH ** -0.5 * log2e)

    def load_y(idx):
        r0 = pl.multiple_of(idx * SEG, SEG)
        return jnp.concatenate([y_v[jj, pl.ds(r0, SEG), :] for jj in range(NSLAB)], axis=1)

    def wt(m, h):
        return pltpu.bitcast(wbuf[widx(m, h)], BF16)

    def filler(seg):
        rn = pl.multiple_of(seg * SEG, SEG)
        tok1 = _ln(x_v[pl.ds(rn, SEG), :].astype(F32)).astype(BF16)
        for h in range(NF):
            for m in range(3):
                q1_s[h * 3 + m] = _mm(tok1, wt(m, h)).astype(BF16)
        h_s[pl.ds(0, 32), :] = tok1

    def attention(kind):
        r0, r1 = {"first": (0, 48), "mid": (0, 80), "last": (32, 80)}[kind]
        R = r1 - r0
        H = h_s[pl.ds(r0, R), :]
        bias = biasl_s[...] if kind == "last" else bias_s[pl.ds(0, R), :]
        valid = bias > np.float32(-1.0)
        g_sz = NH if kind == "first" else G
        nf = NF if kind == "mid" else 0
        if nf:
            HB = h_s[pl.ds(32, 48), :]
        qkv, P, L, O = {}, {}, {}, {}
        acc = [None] * NSLAB
        zpad = jnp.zeros((128 - R, DH), BF16)

        def do_qkv(h):
            if h < nf:
                qkv[h] = tuple(jnp.concatenate([q1_s[h * 3 + m], _mm(HB, wt(m, h)).astype(BF16)], axis=0)
                               for m in range(3))
            else:
                qkv[h] = tuple(_mm(H, wt(m, h)).astype(BF16) for m in range(3))

        def do_s(h):
            q, k, v = qkv[h]
            sc = _mm_nt(q, jnp.concatenate([k, zpad], axis=0))
            t = jnp.where(valid, sc * cscale, bias)
            mx = jnp.max(t, axis=-1, keepdims=True)
            e = jnp.exp2(t - mx)
            L[h] = jnp.sum(e, axis=-1, keepdims=True)
            P[h] = e.astype(BF16)

        def do_pv(h):
            v = qkv[h][2]
            o = _mm(P[h], jnp.concatenate([v, zpad], axis=0))
            O[h] = (o * _recip(L[h])).astype(BF16)

        def do_wo(g):
            if kind == "first" and g == 0:
                wo_cp.wait()
                xb_cp.start()
            og = jnp.concatenate([O[h] for h in range(g * g_sz, (g + 1) * g_sz)], axis=1)
            for n in range(NSLAB):
                wo_n = pltpu.bitcast(wo_v[pl.ds(g * g_sz * 64, g_sz * 64), pl.ds(n * 128, 128)], BF16)
                r = _mm(og, wo_n)
                acc[n] = r if acc[n] is None else acc[n] + r

        NG = NH // g_sz
        done_wo = 0
        for h in range(NH + LAG_PV + 1):
            if h < NH:
                do_qkv(h)
            if LAG_S <= h < NH + LAG_S:
                do_s(h - LAG_S)
            if LAG_PV <= h < NH + LAG_PV:
                do_pv(h - LAG_PV)
            while done_wo < NG and (done_wo + 1) * g_sz - 1 + LAG_PV + LAG_WO <= h:
                do_wo(done_wo)
                done_wo += 1
        while done_wo < NG:
            do_wo(done_wo)
            done_wo += 1
        return acc

    def l2_epilogue(a2, seg):
        x2 = _rb(x1p_s[...] + _rb(a2))
        res = x2 + _rb(_rb(_ln(x2)) * load_y(seg))
        r = pl.multiple_of(seg * SEG, SEG)
        out_v[pl.ds(r, SEG), :] = res.astype(BF16)

    def out_copy(seg):
        r = pl.multiple_of(seg * SEG, SEG)
        return pltpu.make_async_copy(out_v.at[pl.ds(r, SEG), :], out_hbm.at[pl.ds(r, SEG), :], sem_out.at[0])

    def l1_epilogue(a1, seg):
        r1 = pl.multiple_of(seg * SEG, SEG)
        x1 = _rb(x_v[pl.ds(r1, SEG), :].astype(F32) + _rb(a1))
        x1p = _rb(x1 + _rb(_rb(_ln(x1)) * load_y(seg)))
        x1p_s[...] = x1p
        h_s[pl.ds(48, 32), :] = _ln(x1p).astype(BF16)

    mem0 = mem0_v[...]
    h_s[pl.ds(0, 32), :] = _ln(x_v[pl.ds(0, SEG), :].astype(F32)).astype(BF16)
    h_s[pl.ds(32, 16), :] = jnp.concatenate([mem0, mem0], axis=0)
    acc = attention("first")
    filler(1)
    accf = jnp.concatenate(acc, axis=1)
    l1_epilogue(accf[0:32], 0)
    h_s[pl.ds(32, 16), :] = jnp.concatenate([accf[32:40].astype(BF16), mem0], axis=0)

    def step(i, carry):
        acc = attention("mid")
        filler(jnp.minimum(i + 1, NSEG - 1))
        accf = jnp.concatenate(acc, axis=1)
        l2_epilogue(accf[48:80], i - 1)
        l1_epilogue(accf[0:32], i)
        h_s[pl.ds(32, 16), :] = accf[32:48].astype(BF16)
        out_copy(i - 1).start()

        @pl.when(i == 2)
        def _():
            xb_cp.wait()

        return carry

    NST = NSEG
    lax.fori_loop(1, NST, step, 0)
    if NST <= 2:
        xb_cp.wait()

    acc = attention("last")
    accf = jnp.concatenate(acc, axis=1)
    l2_epilogue(accf[16:48], NST - 1)
    out_copy(NST - 1).start()

    def wait_body(i, carry):
        out_copy(i).wait()
        return carry

    lax.fori_loop(0, NST, wait_body, 0)


@functools.partial(jax.jit, static_argnames=("A_seg_len",))
def pallas_interleave_layers__memory_aug_recurrent_mem_tr__ssm_conv_h3__prompt_kernel(
    A_x, A_mem0, A_Wq, A_Wk, A_Wv, A_Wo, A_seg_len, B_q, B_k, B_v, B_shift_k, B_ssm_k, B_ssm_D,
):
    del B_q
    assert A_seg_len == SEG
    x = A_x.reshape(S_LEN, DM)
    mem0 = A_mem0.reshape(MEM, DM)
    wq = A_Wq.reshape(DM // 2, 2 * NH, DH)
    wk = A_Wk.reshape(DM // 2, 2 * NH, DH)
    wv = A_Wv.reshape(DM // 2, 2 * NH, DH)
    wo = A_Wo.reshape(NH * DH, DM)
    k = B_k.reshape(S_LEN, DM)
    v = B_v.reshape(S_LEN, DM)
    ftab = jnp.asarray(_FTAB_U32)
    any_spec = pl.BlockSpec(memory_space=pl.ANY)
    V = pltpu.VMEM
    DMA = pltpu.SemaphoreType.DMA
    scratch = [
        V((S_LEN, DM), BF16),
        V((MEM, DM), BF16),
        V((96, DM // 2, DH), U32),
        V((NH * DH // 2, DM), U32),
        V((NSLAB, S_LEN, 128), BF16),
        V((NSLAB, S_LEN, 128), BF16),
        V((DM, 4), BF16),
        V((NSLAB, 128, S_LEN), BF16),
        V((DM,), BF16),
        V((64, 64, 128), U32),
        V((8, DM), F32),
        V((8 + S_LEN, 128), F32),
        V((S_LEN, 128), F32),
        V((S_LEN, 128), F32),
        V((32, 128, 128), BF16),
        V((32, 128, 128), BF16),
        V((32, 128, 128), F32),
        V((32, 128, 128), F32),
        V((S_LEN, 128), F32),
        V((NSLAB + 1, S_LEN, 128), F32),
        V((S_LEN, DM), BF16),
        V((ROWS, DM), BF16),
        V((12, SEG, DH), BF16),
        V((SEG, DM), F32),
        V((ROWS, 128), F32),
        V((48, 128), F32),
        DMA((1,)), DMA((NSLAB,)), DMA((2,)), DMA((1,)), DMA((1,)), DMA((1,)),
    ]
    out = pl.pallas_call(
        _kernel,
        out_shape=jax.ShapeDtypeStruct((S_LEN, DM), BF16),
        in_specs=[any_spec] * 12,
        out_specs=any_spec,
        scratch_shapes=scratch,
        compiler_params=pltpu.CompilerParams(vmem_limit_bytes=100 * 1024 * 1024),
    )(x, mem0, wq, wk, wv, wo, k, v, B_shift_k, B_ssm_k, B_ssm_D, ftab)
    return out.reshape(1, S_LEN, DM)
```

```python
import functools

import numpy as np
import ml_dtypes

import jax
import jax.numpy as jnp
from jax import lax
import jax.experimental.pallas as pl
import jax.experimental.pallas.tpu as pltpu

F32 = jnp.float32
BF16 = jnp.bfloat16
U32 = jnp.uint32

S_LEN = 2048
DM = 640
NH = 32
DH = 128
MEM = 8
SEG = 32
NSEG = S_LEN // SEG
ROWS = 2 * (MEM + SEG)
NSLAB = DM // 128

_NFFT = 2 * S_LEN


def _build_fft_tables():
    n1 = np.zeros(128, np.int64)
    ri = np.zeros(128, np.int64)
    for g in range(8):
        for r in range(2):
            for nl in range(8):
                c = g * 16 + r * 8 + nl
                n1[c] = 8 * g + nl
                ri[c] = r
    fwd = np.zeros((32, 128, 128), np.float64)
    inv = np.zeros((32, 128, 128), np.float64)
    k1 = np.arange(64)
    q_of = n1
    r_of = ri
    for s in range(1, 32):
        ang = -2.0 * np.pi * (n1[None, :] * (s + 64 * k1[:, None])) / _NFFT
        tre, tim = np.cos(ang), np.sin(ang)
        fwd[s, :64] = np.where(ri[None, :] == 0, tre, -tim)
        fwd[s, 64:] = np.where(ri[None, :] == 0, tim, tre)
        nn = np.arange(64)
        ang = 2.0 * np.pi * (nn[:, None] * (s + 64 * q_of[None, :])) / _NFFT
        ure, uim = np.cos(ang) * (2.0 / _NFFT), np.sin(ang) * (2.0 / _NFFT)
        inv[s, :64] = np.where(r_of[None, :] == 0, ure, -uim)
        inv[s, 64:] = np.where(r_of[None, :] == 0, uim, ure)
    f0 = np.zeros((128, 128), np.float64)
    for c in range(128):
        n = n1[c]
        if ri[c] == 0:
            for q in range(32):
                f0[q, c] = np.cos(2 * np.pi * n * q / 64)
                f0[64 + q, c] = (-1.0) ** n if q == 0 else -np.sin(2 * np.pi * n * q / 64)
        else:
            for q in range(32, 64):
                a = -2.0 * np.pi * n * (32 + 64 * (q - 32)) / _NFFT
                f0[q, c] = np.cos(a)
                f0[64 + q, c] = np.sin(a)
    fwd[0] = f0
    g0 = np.zeros((128, 128), np.float64)
    for c in range(128):
        q, r = q_of[c], r_of[c]
        for n in range(64):
            if q < 32:
                if q == 0:
                    g0[n, c] = (1.0 if r == 0 else (-1.0) ** n) / _NFFT
                else:
                    a = 2 * np.pi * n * q / 64
                    g0[n, c] = 2.0 * (np.cos(a) if r == 0 else -np.sin(a)) / _NFFT
            else:
                a = 2.0 * np.pi * n * (32 + 64 * (q - 32)) / _NFFT
                g0[64 + n, c] = 2.0 * (np.cos(a) if r == 0 else -np.sin(a)) / _NFFT
    inv[0] = g0
    return fwd, inv


_FWD64, _INV64 = _build_fft_tables()
_FWD_BF = _FWD64.astype(np.float32).astype(ml_dtypes.bfloat16)
_INV_BF = _INV64.astype(np.float32).astype(ml_dtypes.bfloat16)


class _SV:
    __slots__ = ("x", "s")

    def __init__(self, x, s=1):
        self.x = x
        self.s = s

    def __neg__(self):
        return _SV(self.x, -self.s)

    def __add__(self, o):
        if o is None:
            return self
        if self.s == o.s:
            return _SV(self.x + o.x, self.s)
        if self.s > 0:
            return _SV(self.x - o.x, 1)
        return _SV(o.x - self.x, 1)

    def __sub__(self, o):
        if o is None:
            return self
        return self + (-o)

    def scale(self, c):
        return _SV(self.x * np.float32(c * self.s), 1)

    def get(self):
        return self.x if self.s > 0 else -self.x


def _cfft(re, im, n, sgn):
    if n == 1:
        return re, im
    er, ei = _cfft(re[0::2], im[0::2], n // 2, sgn)
    orr, oi = _cfft(re[1::2], im[1::2], n // 2, sgn)
    outr = [None] * n
    outi = [None] * n
    h = float(np.sqrt(0.5))
    for k in range(n // 2):
        a, b = orr[k], oi[k]
        if k == 0:
            tr, ti = a, b
        elif 4 * k == n:
            tr, ti = (-b, a) if sgn > 0 else (b, -a)
        elif 8 * k == n:
            if sgn < 0:
                tr, ti = (a + b).scale(h), (b - a).scale(h)
            else:
                tr, ti = (a - b).scale(h), (a + b).scale(h)
        elif 8 * k == 3 * n:
            if sgn < 0:
                tr, ti = (b - a).scale(h), (a + b).scale(-h)
            else:
                tr, ti = (a + b).scale(-h), (a - b).scale(h)
        else:
            ang = sgn * 2 * np.pi * k / n
            c, s = float(np.cos(ang)), float(np.sin(ang))
            tr = a.scale(c) - b.scale(s)
            ti = a.scale(s) + b.scale(c)
        outr[k] = er[k] + tr
        outi[k] = ei[k] + ti
        outr[k + n // 2] = er[k] - tr
        outi[k + n // 2] = ei[k] - ti
    return outr, outi


def _odft(u):
    n = len(u)
    if n == 1:
        return [u[0]], [None]
    h = n // 2
    cr, ci = [], []
    for m in range(h):
        a, b = u[m], u[m + h]
        if m == 0:
            cr.append(a)
            ci.append(-b)
        else:
            ang = -2 * np.pi * m / (2 * n)
            c, s = float(np.cos(ang)), float(np.sin(ang))
            if 8 * m == 2 * n:
                hh = float(np.sqrt(0.5))
                cr.append((a - b).scale(hh))
                ci.append((a + b).scale(-hh))
            else:
                cr.append(a.scale(c) + b.scale(s))
                ci.append(a.scale(s) - b.scale(c))
    Cr, Ci = _cfft(cr, ci, h, -1)
    outr = [None] * h
    outi = [None] * h
    for j in range(h):
        if j % 2 == 0:
            outr[j], outi[j] = Cr[j // 2], Ci[j // 2]
        else:
            l = (j - 1) // 2
            outr[j], outi[j] = Cr[h - 1 - l], -Ci[h - 1 - l]
    return outr, outi


def _rdft(x):
    n = len(x)
    if n == 1:
        return [x[0]], [None]
    h = n // 2
    er, ei = _rdft([x[i] + x[i + h] for i in range(h)])
    orr, oi = _odft([x[i] - x[i + h] for i in range(h)])
    outr = [None] * (h + 1)
    outi = [None] * (h + 1)
    for k in range(h + 1):
        if k % 2 == 0:
            outr[k], outi[k] = er[k // 2], ei[k // 2]
        else:
            outr[k], outi[k] = orr[k // 2], oi[k // 2]
    return outr, outi


def _paddft(x):
    n = len(x)
    er, ei = _rdft(x)
    orr, oi = _odft(x)
    outr = [None] * (n + 1)
    outi = [None] * (n + 1)
    for k in range(n + 1):
        if k % 2 == 0:
            outr[k], outi[k] = er[k // 2], ei[k // 2]
        else:
            outr[k], outi[k] = orr[k // 2], oi[k // 2]
    return outr, outi


def _odft_T(sr, si):
    h = len(sr)
    n = 2 * h
    Cr = [None] * h
    Ci = [None] * h
    for j in range(h):
        if j % 2 == 0:
            Cr[j // 2], Ci[j // 2] = sr[j], si[j]
        else:
            l = (j - 1) // 2
            Cr[h - 1 - l], Ci[h - 1 - l] = sr[j], -si[j]
    cr, ci = _cfft(Cr, Ci, h, +1)
    lo, hi = [], []
    for m in range(h):
        if m == 0:
            lo.append(cr[0])
            hi.append(-ci[0])
        else:
            ang = -2 * np.pi * m / (2 * n)
            c, s = float(np.cos(ang)), float(np.sin(ang))
            if 8 * m == 2 * n:
                hh = float(np.sqrt(0.5))
                lo.append((cr[m] - ci[m]).scale(hh))
                hi.append((cr[m] + ci[m]).scale(-hh))
            else:
                lo.append(cr[m].scale(c) + ci[m].scale(s))
                hi.append(cr[m].scale(s) - ci[m].scale(c))
    return lo + hi


def _rdft_T(sr, si):
    h = len(sr) - 1
    if h == 0:
        return [sr[0]]
    ev_r, ev_i = sr[0::2], si[0::2]
    od_r, od_i = sr[1::2], si[1::2]
    s = _rdft_T(ev_r, ev_i)
    if h == 1:
        d = [od_r[0]]
    else:
        d = _odft_T(od_r, od_i)
    return [s[i] + d[i] for i in range(h)] + [s[i] - d[i] for i in range(h)]


def _paddft_T(sr, si):
    n = len(sr) - 1
    a = _rdft_T(sr[0::2], si[0::2])
    b = _odft_T(sr[1::2], si[1::2])
    return [a[i] + b[i] for i in range(n)]


def _mm(a, b):
    return jnp.dot(a, b, preferred_element_type=F32)


def _mm_nt(a, b):
    return lax.dot_general(a, b, (((1,), (1,)), ((), ())), preferred_element_type=F32)


def _ln(x):
    m = jnp.mean(x, axis=-1, keepdims=True)
    d = x - m
    v = jnp.mean(d * d, axis=-1, keepdims=True)
    return d * lax.rsqrt(v + np.float32(1e-5))


def _rb(x):
    return x.astype(BF16).astype(F32)


def _recip(l):
    r = pl.reciprocal(l, approx=True)
    return r * (np.float32(2.0) - l * r)


def _build_seed_table():
    c = np.arange(128)
    n1 = (c // 16) * 8 + (c % 8)
    k = np.arange(64)
    tab = np.zeros((648, 128), np.float64)
    th = -2.0 * np.pi * (n1[None, :] * k[:, None]) / 64.0
    tab[0:64], tab[64:128] = np.cos(th), np.sin(th)
    th = 2.0 * np.pi * (k[:, None] * n1[None, :]) / 64.0
    tab[128:192], tab[192:256] = np.cos(th) * (2.0 / _NFFT), np.sin(th) * (2.0 / _NFFT)
    dl = 2.0 * np.pi * k / _NFFT
    tab[256:320], tab[320:384] = np.cos(dl)[:, None], np.sin(dl)[:, None]
    dl = -2.0 * np.pi * n1 / _NFFT
    tab[384], tab[385] = np.cos(dl), np.sin(dl)
    tab[392:520] = _FWD64[0]
    tab[520:648] = _INV64[0]
    return tab.astype(np.float32)


_SEED_TAB = _build_seed_table()


def _kernel(x_hbm, mem0_hbm, wq_hbm, wk_hbm, wv_hbm, wo_hbm, k_hbm, v_hbm, shift_hbm,
            ssmk_hbm, ssmd_hbm, seed_hbm,
            out_hbm,
            x_v, mem0_v, wbuf, wo_v, k_v, v_v, shift_v, ssmk_v, ssmd_v, seed_v, ffw_s, fiv_s, wrow_s,
            kf_s, kv_s, ht_s, akv_s, ah_s, ba_s, bb_s, ta_s, y_v, out_v, h_s, q1_s, x1p_s, bias_s, biasl_s,
            sem_f, sem_s, sem_x, sem_w, sem_wo, sem_out):
    def slab_copies(j):
        return [pltpu.make_async_copy(k_hbm.at[:, pl.ds(j * 128, 128)], k_v.at[j], sem_s.at[j]),
                pltpu.make_async_copy(v_hbm.at[:, pl.ds(j * 128, 128)], v_v.at[j], sem_s.at[j]),
                pltpu.make_async_copy(ssmk_hbm.at[pl.ds(j * 128, 128), :], ssmk_v.at[j], sem_s.at[j])]

    f_cps = [pltpu.make_async_copy(shift_hbm, shift_v, sem_f.at[0]),
             pltpu.make_async_copy(ssmd_hbm, ssmd_v, sem_f.at[0]),
             pltpu.make_async_copy(seed_hbm, seed_v, sem_f.at[0])]
    XA = 4 * SEG
    xa_cps = [pltpu.make_async_copy(x_hbm.at[pl.ds(0, XA), :], x_v.at[pl.ds(0, XA), :], sem_x.at[0]),
              pltpu.make_async_copy(mem0_hbm, mem0_v, sem_x.at[0])]
    xb_cp = pltpu.make_async_copy(x_hbm.at[pl.ds(XA, S_LEN - XA), :], x_v.at[pl.ds(XA, S_LEN - XA), :],
                                  sem_x.at[1])
    w_cps = []
    for m, w_hbm in enumerate((wq_hbm, wk_hbm, wv_hbm)):
        w32 = w_hbm.bitcast(U32)
        for j in range(32):
            w_cps.append(pltpu.make_async_copy(w32.at[:, j, :], wbuf.at[m * 32 + j], sem_w.at[0]))
    wo_cp = pltpu.make_async_copy(wo_hbm.bitcast(U32), wo_v, sem_wo.at[0])

    for c in f_cps + slab_copies(0) + slab_copies(1):
        c.start()

    r_i = lax.broadcasted_iota(jnp.int32, (ROWS, 128), 0)
    c_i = lax.broadcasted_iota(jnp.int32, (ROWS, 128), 1)
    same = jnp.logical_and((r_i < 40) == (c_i < 40), c_i < ROWS)
    memr = jnp.logical_and(r_i >= 32, r_i < 48)
    memc = jnp.logical_and(c_i >= 32, c_i < 48)
    ok = jnp.logical_or(jnp.logical_or(memr, memc), c_i <= r_i)
    log2e = float(np.log2(np.e))
    bias_s[...] = jnp.where(same, jnp.where(ok, np.float32(0.0), np.float32(-1e9 * log2e)),
                            np.float32(-1e30))
    r_l = lax.broadcasted_iota(jnp.int32, (48, 128), 0) + 32
    c_l = lax.broadcasted_iota(jnp.int32, (48, 128), 1) + 32
    same_l = jnp.logical_and((r_l < 40) == (c_l < 40), c_l < ROWS)
    ok_l = jnp.logical_or(jnp.logical_or(r_l < 48, c_l < 48), c_l <= r_l)
    biasl_s[...] = jnp.where(same_l, jnp.where(ok_l, np.float32(0.0), np.float32(-1e9 * log2e)),
                             np.float32(-1e30))
    kf_s[pl.ds(0, 8), :] = jnp.zeros((8, 128), F32)

    def zero_b(i, c):
        bb_s[i] = jnp.zeros((128, 128), F32)
        return c


    for c in f_cps:
        c.wait()
    ri0 = (lax.broadcasted_iota(jnp.int32, (64, 128), 1) // 8) % 2 == 0
    ffw_s[0] = pltpu.bitcast(seed_v[pl.ds(392, 128), :].astype(BF16), U32)
    fiv_s[0] = pltpu.bitcast(seed_v[pl.ds(520, 128), :].astype(BF16), U32)
    cdf, sdf = seed_v[pl.ds(384, 1), :], seed_v[pl.ds(385, 1), :]

    def gen_fwd(sl, cs):
        c0, s0 = cs
        c1 = c0 * cdf - s0 * sdf
        s1 = s0 * cdf + c0 * sdf
        top = jnp.where(ri0, c1, -s1)
        bot = jnp.where(ri0, s1, c1)
        ffw_s[sl] = pltpu.bitcast(jnp.concatenate([top, bot], axis=0).astype(BF16), U32)
        return c1, s1

    lax.fori_loop(1, 32, gen_fwd, (seed_v[pl.ds(0, 64), :], seed_v[pl.ds(64, 64), :]))

    def gen_inv(sl, cs):
        c0, s0 = cs
        cd, sd = seed_v[pl.ds(256, 64), :], seed_v[pl.ds(320, 64), :]
        c1 = c0 * cd - s0 * sd
        s1 = s0 * cd + c0 * sd
        top = jnp.where(ri0, c1, -s1)
        bot = jnp.where(ri0, s1, c1)
        fiv_s[sl] = pltpu.bitcast(jnp.concatenate([top, bot], axis=0).astype(BF16), U32)
        return c1, s1

    lax.fori_loop(1, 32, gen_inv, (seed_v[pl.ds(128, 64), :], seed_v[pl.ds(192, 64), :]))

    for c in slab_copies(0) + slab_copies(1):
        c.wait()
    NPRE = 6
    for c in slab_copies(2) + slab_copies(3) + slab_copies(4) + xa_cps + w_cps[:NPRE]:
        c.start()
    wrow_s[pl.ds(0, 4), :] = shift_v[...].astype(F32)
    wrow_s[pl.ds(4, 1), :] = ssmd_v[...].astype(F32).reshape(1, DM)
    row0 = lax.broadcasted_iota(jnp.int32, (8, 128), 0) == 0
    RB = 128

    def taps(j):
        lane0 = j * 128
        return ([wrow_s[pl.ds(t, 1), pl.ds(lane0, 128)] for t in range(4)],
                wrow_s[pl.ds(4, 1), pl.ds(lane0, 128)])

    def prep_p(j, r, n):
        kf_s[pl.ds(8 + r, n), :] = k_v[j, pl.ds(r, n), :].astype(F32)

    def prep_q(j, r, w):
        ks = (kf_s[pl.ds(8 + r, RB), :] * w[0] + kf_s[pl.ds(7 + r, RB), :] * w[1]
              + kf_s[pl.ds(6 + r, RB), :] * w[2] + kf_s[pl.ds(5 + r, RB), :] * w[3])
        kv_s[pl.ds(r, RB), :] = ks * v_v[j, pl.ds(r, RB), :].astype(F32)

    def prep_t(j, dd):
        ht = ssmk_v[j].astype(F32).T
        ht_s[pl.ds(8, S_LEN - 8), :] = ht[8:]
        ht_s[pl.ds(0, 8), :] = ht[:8] + jnp.where(row0, dd, np.float32(0.0))

    def pk(re, im):
        return jnp.concatenate([re, im], axis=0).astype(BF16)

    def fwd_nets(src, dst):
        def fwd_a(g, c):
            r = pl.multiple_of(g * 8, 8)
            r2 = pl.multiple_of(g * 16, 16)
            xs = [_SV(src[pl.ds(n2 * 64 + r, 8), :]) for n2 in range(32)]
            orr, oi = _odft(xs)
            for q in range(16):
                dst[2 * q + 1, pl.ds(r2, 16), :] = pk(orr[q].get(), oi[q].get())
            return c

        def fwd_b(g, c):
            r = pl.multiple_of(g * 8, 8)
            r2 = pl.multiple_of(g * 16, 16)
            xs = [_SV(src[pl.ds(n2 * 64 + r, 8), :]) for n2 in range(32)]
            er, ei = _rdft(xs)
            dst[0, pl.ds(r2, 16), :] = pk(er[0].get(), er[16].get())
            for q in range(1, 16):
                dst[2 * q, pl.ds(r2, 16), :] = pk(er[q].get(), ei[q].get())
            return c

        lax.fori_loop(0, 8, fwd_a, 0)
        lax.fori_loop(0, 8, fwd_b, 0)

    def inv_a(br, r):
        sr = [_SV(br[2 * q + 1, pl.ds(r, 8), :]) for q in range(16)]
        si = [_SV(br[2 * q + 1, pl.ds(64 + r, 8), :]) for q in range(16)]
        bb = _odft_T(sr, si)
        for n2 in range(32):
            ta_s[pl.ds(n2 * 64 + r, 8), :] = bb[n2].get()

    def inv_b(br, jy, r):
        sr = [None] * 17
        si = [None] * 17
        sr[0] = _SV(br[0, pl.ds(r, 8), :])
        sr[16] = _SV(br[0, pl.ds(64 + r, 8), :])
        for q in range(1, 16):
            sr[q] = _SV(br[2 * q, pl.ds(r, 8), :])
            si[q] = _SV(br[2 * q, pl.ds(64 + r, 8), :])
        aa = _rdft_T(sr, si)
        for n2 in range(32):
            prev = _SV(ta_s[pl.ds(n2 * 64 + r, 8), :])
            y_v[jy, pl.ds(n2 * 64 + r, 8), :] = (aa[n2] + prev).get()

    def mxu_block(j, bw, br):
        jn = j + 1
        jy = j - 1
        do_prep = j + 1 < NSL
        do_inv = j >= 1
        w, dd = taps(min(jn, NSLAB - 1))
        LAG = 3
        X, Y = {}, {}
        for t in range(32 + LAG):
            if do_prep and t % 8 == 0 and t < 32:
                nb = t // 2
                ht_s[pl.ds(nb * 128, 512), :] = ssmk_v[jn, :, pl.ds(nb * 128, 512)].astype(F32).T
            if do_prep and t % 2 == 0 and t < 32:
                prep_p(jn, (t // 2) * RB, RB)
            if do_prep and t % 2 == 1 and t < 32:
                prep_q(jn, (t // 2) * RB, w)
            if do_inv and t % 4 == 0 and t < 32:
                inv_a(br, (t // 4) * 8)
            if do_inv and t % 4 == 2 and t < 32:
                inv_b(br, jy, (t // 4) * 8)
            if t < 32:
                f = pltpu.bitcast(ffw_s[t], BF16)
                X[t] = (_mm(f, akv_s[t]), _mm(f, ah_s[t]))
            if 1 <= t <= 32:
                sl = t - 1
                xk, xh = X.pop(sl)
                kr, ki, hr, hi = xk[:64], xk[64:], xh[:64], xh[64:]
                yr = kr * hr - ki * hi
                yi = kr * hi + ki * hr
                if sl == 0:
                    yr = jnp.concatenate([jnp.where(row0, kr[:8] * hr[:8], yr[:8]), yr[8:]], axis=0)
                    yi = jnp.concatenate([jnp.where(row0, ki[:8] * hi[:8], yi[:8]), yi[8:]], axis=0)
                parts = []
                for jj in range(8):
                    parts.append(yr[8 * jj:8 * jj + 8])
                    parts.append(yi[8 * jj:8 * jj + 8])
                Y[sl] = jnp.concatenate(parts, axis=0).astype(BF16)
            if t >= LAG:
                sl = t - LAG
                bw[sl] = _mm(pltpu.bitcast(fiv_s[sl], BF16), Y.pop(sl))
        if do_prep:
            ht_s[pl.ds(0, 8), :] = ht_s[pl.ds(0, 8), :] + jnp.where(row0, dd, np.float32(0.0))

    NSL = NSLAB
    w0, dd0 = taps(0)

    def p_body(b, c):
        prep_p(0, pl.multiple_of(b * 256, 256), 256)
        return c

    lax.fori_loop(0, S_LEN // 256, p_body, 0)

    def q_body(b, c):
        prep_q(0, pl.multiple_of(b * RB, RB), w0)
        return c

    lax.fori_loop(0, S_LEN // RB, q_body, 0)
    prep_t(0, dd0)

    NSL = NSLAB

    for j in range(NSL):
        fwd_nets(kv_s, akv_s)
        fwd_nets(ht_s, ah_s)
        if j == 1:
            for c in slab_copies(2) + slab_copies(3) + slab_copies(4) + xa_cps:
                c.wait()
            for c in w_cps[NPRE:]:
                c.start()
            if 1:
                wo_cp.start()
        mxu_block(j, (ba_s, bb_s)[j % 2], (ba_s, bb_s)[1 - j % 2])
    jl = NSL - 1

    def ia_body(g, c):
        inv_a(ba_s if jl % 2 == 0 else bb_s, pl.multiple_of(g * 8, 8))
        return c

    def ib_body(g, c):
        inv_b(ba_s if jl % 2 == 0 else bb_s, jl, pl.multiple_of(g * 8, 8))
        return c

    lax.fori_loop(0, 8, ia_body, 0)
    lax.fori_loop(0, 8, ib_body, 0)

    for c in w_cps:
        c.wait()
    if not 1:
        wo_cp.start()

    def relayout_pair(p):
        for m in range(3):
            ia = m * 32 + p
            ib = ia + 16
            for r in range(0, 320, 64):
                a = wbuf[ia, pl.ds(r, 64), :]
                b = wbuf[ib, pl.ds(r, 64), :]
                wbuf[ia, pl.ds(r, 64), :] = (a & np.uint32(0xFFFF)) | (b << 16)
                wbuf[ib, pl.ds(r, 64), :] = (a >> 16) | (b & np.uint32(0xFFFF0000))

    def widx(m, h):
        return m * 32 + (h % 2) * 16 + h // 2

    NF = 4
    G = 8
    LAGS_MID = (3, 6, 6)
    LAGS_EDGE = (4, 7, 6)
    cscale = np.float32(DH ** -0.5 * log2e)

    def load_y(idx):
        r0 = pl.multiple_of(idx * SEG, SEG)
        return jnp.concatenate([y_v[jj, pl.ds(r0, SEG), :] for jj in range(NSLAB)], axis=1)

    def wt(m, h):
        return pltpu.bitcast(wbuf[widx(m, h)], BF16)

    def filler(seg):
        rn = pl.multiple_of(seg * SEG, SEG)
        tok1 = _ln(x_v[pl.ds(rn, SEG), :].astype(F32)).astype(BF16)
        for h in range(NF):
            for m in range(3):
                q1_s[h * 3 + m] = _mm(tok1, wt(m, h)).astype(BF16)
        h_s[pl.ds(0, 32), :] = tok1

    def attention(kind):
        r0, r1 = {"first": (0, 48), "mid": (0, 80), "last": (32, 80)}[kind]
        R = r1 - r0
        H = h_s[pl.ds(r0, R), :]
        bias = biasl_s[...] if kind == "last" else bias_s[pl.ds(0, R), :]
        valid = bias > np.float32(-1.0)
        g_sz = NH if kind == "first" else G
        nf = NF if kind == "mid" else 0
        if nf:
            HB = h_s[pl.ds(32, 48), :]
        qkv, P, L, O = {}, {}, {}, {}
        acc = [None] * NSLAB
        zpad = jnp.zeros((128 - R, DH), BF16)

        def do_qkv(h):
            if h < nf:
                qkv[h] = tuple(jnp.concatenate([q1_s[h * 3 + m], _mm(HB, wt(m, h)).astype(BF16)], axis=0)
                               for m in range(3))
            else:
                qkv[h] = tuple(_mm(H, wt(m, h)).astype(BF16) for m in range(3))

        def do_s(h):
            q, k, v = qkv[h]
            sc = _mm_nt(q, jnp.concatenate([k, zpad], axis=0))
            t = jnp.where(valid, sc * cscale, bias)
            mx = jnp.max(t, axis=-1, keepdims=True)
            e = jnp.exp2(t - mx)
            L[h] = jnp.sum(e, axis=-1, keepdims=True)
            P[h] = e.astype(BF16)

        def do_pv(h):
            v = qkv[h][2]
            o = _mm(P[h], jnp.concatenate([v, zpad], axis=0))
            O[h] = (o * _recip(L[h])).astype(BF16)

        def do_wo(g):
            if kind == "first" and g == 0:
                wo_cp.wait()
                xb_cp.start()
            og = jnp.concatenate([O[h] for h in range(g * g_sz, (g + 1) * g_sz)], axis=1)
            for n in range(NSLAB):
                wo_n = pltpu.bitcast(wo_v[pl.ds(g * g_sz * 64, g_sz * 64), pl.ds(n * 128, 128)], BF16)
                r = _mm(og, wo_n)
                acc[n] = r if acc[n] is None else acc[n] + r

        NG = NH // g_sz
        done_wo = 0
        LAG_S, LAG_PV, LAG_WO = LAGS_MID if kind == "mid" else LAGS_EDGE
        for h in range(NH + LAG_PV + 1):
            if kind == "first" and h % 2 == 0:
                if h == 0:
                    relayout_pair(0)
                if h + 2 < NH:
                    relayout_pair(h // 2 + 1)
            if h < NH:
                do_qkv(h)
            if LAG_S <= h < NH + LAG_S:
                do_s(h - LAG_S)
            if LAG_PV <= h < NH + LAG_PV:
                do_pv(h - LAG_PV)
            while done_wo < NG and (done_wo + 1) * g_sz - 1 + LAG_PV + LAG_WO <= h:
                do_wo(done_wo)
                done_wo += 1
        while done_wo < NG:
            do_wo(done_wo)
            done_wo += 1
        return acc

    def l2_epilogue(a2, seg):
        x2 = _rb(x1p_s[...] + _rb(a2))
        res = x2 + _rb(_rb(_ln(x2)) * load_y(seg))
        r = pl.multiple_of(seg * SEG, SEG)
        out_v[pl.ds(r, SEG), :] = res.astype(BF16)

    def out_copy(seg):
        r = pl.multiple_of(seg * SEG, SEG)
        return pltpu.make_async_copy(out_v.at[pl.ds(r, SEG), :], out_hbm.at[pl.ds(r, SEG), :], sem_out.at[0])

    def l1_epilogue(a1, seg):
        r1 = pl.multiple_of(seg * SEG, SEG)
        x1 = _rb(x_v[pl.ds(r1, SEG), :].astype(F32) + _rb(a1))
        x1p = _rb(x1 + _rb(_rb(_ln(x1)) * load_y(seg)))
        x1p_s[...] = x1p
        h_s[pl.ds(48, 32), :] = _ln(x1p).astype(BF16)

    mem0 = mem0_v[...]
    h_s[pl.ds(0, 32), :] = _ln(x_v[pl.ds(0, SEG), :].astype(F32)).astype(BF16)
    h_s[pl.ds(32, 16), :] = jnp.concatenate([mem0, mem0], axis=0)
    acc = attention("first")
    filler(1)
    accf = jnp.concatenate(acc, axis=1)
    l1_epilogue(accf[0:32], 0)
    h_s[pl.ds(32, 16), :] = jnp.concatenate([accf[32:40].astype(BF16), mem0], axis=0)

    def step(i, carry):
        acc = attention("mid")
        filler(jnp.minimum(i + 1, NSEG - 1))
        accf = jnp.concatenate(acc, axis=1)
        l2_epilogue(accf[48:80], i - 1)
        l1_epilogue(accf[0:32], i)
        h_s[pl.ds(32, 16), :] = accf[32:48].astype(BF16)
        out_copy(i - 1).start()

        @pl.when(i == 2)
        def _():
            xb_cp.wait()

        return carry

    NST = NSEG
    lax.fori_loop(1, NST, step, 0)
    if NST <= 2:
        xb_cp.wait()

    acc = attention("last")
    accf = jnp.concatenate(acc, axis=1)
    l2_epilogue(accf[16:48], NST - 1)
    out_copy(NST - 1).start()

    def wait_body(i, carry):
        out_copy(i).wait()
        return carry

    lax.fori_loop(0, NST, wait_body, 0)


@functools.partial(jax.jit, static_argnames=("A_seg_len",))
def pallas_interleave_layers__memory_aug_recurrent_mem_tr__ssm_conv_h3__prompt_kernel(
    A_x, A_mem0, A_Wq, A_Wk, A_Wv, A_Wo, A_seg_len, B_q, B_k, B_v, B_shift_k, B_ssm_k, B_ssm_D,
):
    del B_q
    assert A_seg_len == SEG
    x = A_x.reshape(S_LEN, DM)
    mem0 = A_mem0.reshape(MEM, DM)
    wq = A_Wq.reshape(DM // 2, 2 * NH, DH)
    wk = A_Wk.reshape(DM // 2, 2 * NH, DH)
    wv = A_Wv.reshape(DM // 2, 2 * NH, DH)
    wo = A_Wo.reshape(NH * DH, DM)
    k = B_k.reshape(S_LEN, DM)
    v = B_v.reshape(S_LEN, DM)
    seed = jnp.asarray(_SEED_TAB)
    any_spec = pl.BlockSpec(memory_space=pl.ANY)
    V = pltpu.VMEM
    DMA = pltpu.SemaphoreType.DMA
    scratch = [
        V((S_LEN, DM), BF16),
        V((MEM, DM), BF16),
        V((96, DM // 2, DH), U32),
        V((NH * DH // 2, DM), U32),
        V((NSLAB, S_LEN, 128), BF16),
        V((NSLAB, S_LEN, 128), BF16),
        V((4, DM), BF16),
        V((NSLAB, 128, S_LEN), BF16),
        V((DM,), BF16),
        V((648, 128), F32),
        V((32, 64, 128), U32),
        V((32, 64, 128), U32),
        V((8, DM), F32),
        V((8 + S_LEN, 128), F32),
        V((S_LEN, 128), F32),
        V((S_LEN, 128), F32),
        V((32, 128, 128), BF16),
        V((32, 128, 128), BF16),
        V((32, 128, 128), F32),
        V((32, 128, 128), F32),
        V((S_LEN, 128), F32),
        V((NSLAB + 1, S_LEN, 128), F32),
        V((S_LEN, DM), BF16),
        V((ROWS, DM), BF16),
        V((12, SEG, DH), BF16),
        V((SEG, DM), F32),
        V((ROWS, 128), F32),
        V((48, 128), F32),
        DMA((1,)), DMA((NSLAB,)), DMA((2,)), DMA((1,)), DMA((1,)), DMA((1,)),
    ]
    out = pl.pallas_call(
        _kernel,
        out_shape=jax.ShapeDtypeStruct((S_LEN, DM), BF16),
        in_specs=[any_spec] * 12,
        out_specs=any_spec,
        scratch_shapes=scratch,
        compiler_params=pltpu.CompilerParams(vmem_limit_bytes=100 * 1024 * 1024),
    )(x, mem0, wq, wk, wv, wo, k, v, B_shift_k.T, B_ssm_k, B_ssm_D, seed)
    return out.reshape(1, S_LEN, DM)
```

```python
import functools

import numpy as np

import jax
import jax.numpy as jnp
from jax import lax
import jax.experimental.pallas as pl
import jax.experimental.pallas.tpu as pltpu

F32 = jnp.float32
BF16 = jnp.bfloat16
U32 = jnp.uint32

S_LEN = 2048
DM = 640
NH = 32
DH = 128
MEM = 8
SEG = 32
NSEG = S_LEN // SEG
ROWS = 2 * (MEM + SEG)
NSLAB = DM // 128
NF = 5

_NFFT = 2 * S_LEN


def _build_slot0_tables():
    c = np.arange(128)
    n1 = (c // 16) * 8 + (c % 8)
    ri = (c // 8) % 2
    f0 = np.zeros((128, 128), np.float64)
    g0 = np.zeros((128, 128), np.float64)
    for col in range(128):
        n = n1[col]
        if ri[col] == 0:
            for q in range(32):
                f0[q, col] = np.cos(2 * np.pi * n * q / 64)
                f0[64 + q, col] = (-1.0) ** n if q == 0 else -np.sin(2 * np.pi * n * q / 64)
        else:
            for q in range(32, 64):
                a = -2.0 * np.pi * n * (32 + 64 * (q - 32)) / _NFFT
                f0[q, col] = np.cos(a)
                f0[64 + q, col] = np.sin(a)
    for col in range(128):
        q, r = n1[col], ri[col]
        for n in range(64):
            if q < 32:
                if q == 0:
                    g0[n, col] = (1.0 if r == 0 else (-1.0) ** n) / _NFFT
                else:
                    a = 2 * np.pi * n * q / 64
                    g0[n, col] = 2.0 * (np.cos(a) if r == 0 else -np.sin(a)) / _NFFT
            else:
                a = 2.0 * np.pi * n * (32 + 64 * (q - 32)) / _NFFT
                g0[64 + n, col] = 2.0 * (np.cos(a) if r == 0 else -np.sin(a)) / _NFFT
    return f0, g0


_FWD0, _INV0 = _build_slot0_tables()


class _SV:
    __slots__ = ("x", "s")

    def __init__(self, x, s=1):
        self.x = x
        self.s = s

    def __neg__(self):
        return _SV(self.x, -self.s)

    def __add__(self, o):
        if o is None:
            return self
        if self.s == o.s:
            return _SV(self.x + o.x, self.s)
        if self.s > 0:
            return _SV(self.x - o.x, 1)
        return _SV(o.x - self.x, 1)

    def __sub__(self, o):
        if o is None:
            return self
        return self + (-o)

    def scale(self, c):
        return _SV(self.x * np.float32(c * self.s), 1)

    def get(self):
        return self.x if self.s > 0 else -self.x


def _cfft(re, im, n, sgn):
    if n == 1:
        return re, im
    er, ei = _cfft(re[0::2], im[0::2], n // 2, sgn)
    orr, oi = _cfft(re[1::2], im[1::2], n // 2, sgn)
    outr = [None] * n
    outi = [None] * n
    h = float(np.sqrt(0.5))
    for k in range(n // 2):
        a, b = orr[k], oi[k]
        if k == 0:
            tr, ti = a, b
        elif 4 * k == n:
            tr, ti = (-b, a) if sgn > 0 else (b, -a)
        elif 8 * k == n:
            if sgn < 0:
                tr, ti = (a + b).scale(h), (b - a).scale(h)
            else:
                tr, ti = (a - b).scale(h), (a + b).scale(h)
        elif 8 * k == 3 * n:
            if sgn < 0:
                tr, ti = (b - a).scale(h), (a + b).scale(-h)
            else:
                tr, ti = (a + b).scale(-h), (a - b).scale(h)
        else:
            ang = sgn * 2 * np.pi * k / n
            c, s = float(np.cos(ang)), float(np.sin(ang))
            tr = a.scale(c) - b.scale(s)
            ti = a.scale(s) + b.scale(c)
        outr[k] = er[k] + tr
        outi[k] = ei[k] + ti
        outr[k + n // 2] = er[k] - tr
        outi[k + n // 2] = ei[k] - ti
    return outr, outi


def _odft(u):
    n = len(u)
    if n == 1:
        return [u[0]], [None]
    h = n // 2
    cr, ci = [], []
    for m in range(h):
        a, b = u[m], u[m + h]
        if m == 0:
            cr.append(a)
            ci.append(-b)
        else:
            ang = -2 * np.pi * m / (2 * n)
            c, s = float(np.cos(ang)), float(np.sin(ang))
            if 8 * m == 2 * n:
                hh = float(np.sqrt(0.5))
                cr.append((a - b).scale(hh))
                ci.append((a + b).scale(-hh))
            else:
                cr.append(a.scale(c) + b.scale(s))
                ci.append(a.scale(s) - b.scale(c))
    Cr, Ci = _cfft(cr, ci, h, -1)
    outr = [None] * h
    outi = [None] * h
    for j in range(h):
        if j % 2 == 0:
            outr[j], outi[j] = Cr[j // 2], Ci[j // 2]
        else:
            l = (j - 1) // 2
            outr[j], outi[j] = Cr[h - 1 - l], -Ci[h - 1 - l]
    return outr, outi


def _rdft(x):
    n = len(x)
    if n == 1:
        return [x[0]], [None]
    h = n // 2
    er, ei = _rdft([x[i] + x[i + h] for i in range(h)])
    orr, oi = _odft([x[i] - x[i + h] for i in range(h)])
    outr = [None] * (h + 1)
    outi = [None] * (h + 1)
    for k in range(h + 1):
        if k % 2 == 0:
            outr[k], outi[k] = er[k // 2], ei[k // 2]
        else:
            outr[k], outi[k] = orr[k // 2], oi[k // 2]
    return outr, outi


def _odft_T(sr, si):
    h = len(sr)
    n = 2 * h
    Cr = [None] * h
    Ci = [None] * h
    for j in range(h):
        if j % 2 == 0:
            Cr[j // 2], Ci[j // 2] = sr[j], si[j]
        else:
            l = (j - 1) // 2
            Cr[h - 1 - l], Ci[h - 1 - l] = sr[j], -si[j]
    cr, ci = _cfft(Cr, Ci, h, +1)
    lo, hi = [], []
    for m in range(h):
        if m == 0:
            lo.append(cr[0])
            hi.append(-ci[0])
        else:
            ang = -2 * np.pi * m / (2 * n)
            c, s = float(np.cos(ang)), float(np.sin(ang))
            if 8 * m == 2 * n:
                hh = float(np.sqrt(0.5))
                lo.append((cr[m] - ci[m]).scale(hh))
                hi.append((cr[m] + ci[m]).scale(-hh))
            else:
                lo.append(cr[m].scale(c) + ci[m].scale(s))
                hi.append(cr[m].scale(s) - ci[m].scale(c))
    return lo + hi


def _rdft_T(sr, si):
    h = len(sr) - 1
    if h == 0:
        return [sr[0]]
    ev_r, ev_i = sr[0::2], si[0::2]
    od_r, od_i = sr[1::2], si[1::2]
    s = _rdft_T(ev_r, ev_i)
    if h == 1:
        d = [od_r[0]]
    else:
        d = _odft_T(od_r, od_i)
    return [s[i] + d[i] for i in range(h)] + [s[i] - d[i] for i in range(h)]


def _mm(a, b):
    return jnp.dot(a, b, preferred_element_type=F32)


def _mm_nt(a, b):
    return lax.dot_general(a, b, (((1,), (1,)), ((), ())), preferred_element_type=F32)


def _ln(x):
    m = jnp.mean(x, axis=-1, keepdims=True)
    d = x - m
    v = jnp.mean(d * d, axis=-1, keepdims=True)
    return d * lax.rsqrt(v + np.float32(1e-5))


def _rb(x):
    return x.astype(BF16).astype(F32)


def _recip(l):
    r = pl.reciprocal(l, approx=True)
    return r * (np.float32(2.0) - l * r)


def _build_seed_table():
    c = np.arange(128)
    n1 = (c // 16) * 8 + (c % 8)
    k = np.arange(64)
    tab = np.zeros((648, 128), np.float64)
    th = -2.0 * np.pi * (n1[None, :] * k[:, None]) / 64.0
    tab[0:64], tab[64:128] = np.cos(th), np.sin(th)
    th = 2.0 * np.pi * (k[:, None] * n1[None, :]) / 64.0
    tab[128:192], tab[192:256] = np.cos(th) * (2.0 / _NFFT), np.sin(th) * (2.0 / _NFFT)
    dl = 2.0 * np.pi * k / _NFFT
    tab[256:320], tab[320:384] = np.cos(dl)[:, None], np.sin(dl)[:, None]
    dl = -2.0 * np.pi * n1 / _NFFT
    tab[384], tab[385] = np.cos(dl), np.sin(dl)
    tab[392:520] = _FWD0
    tab[520:648] = _INV0
    return tab.astype(np.float32)


_SEED_TAB = _build_seed_table()


def _kernel(x_hbm, mem0_hbm, wq_hbm, wk_hbm, wv_hbm, wo_hbm, k_hbm, v_hbm, shift_hbm,
            ssmk_hbm, ssmd_hbm, seed_hbm,
            out_hbm,
            x_v, mem0_v, wbuf, wo_v, k_v, v_v, shift_v, ssmk_v, ssmd_v, seed_v, ffw_s, fiv_s, wrow_s,
            kf_s, kv_s, ht_s, akv_s, ah_s, ba_s, bb_s, ta_s, y_v, out_v, h_s, q1_s, x1p_s, bias_s, biasl_s,
            sem_f, sem_s, sem_x, sem_w, sem_wo, sem_out):
    slab_cps = [[pltpu.make_async_copy(k_hbm.at[:, pl.ds(j * 128, 128)], k_v.at[j], sem_s.at[j]),
                 pltpu.make_async_copy(v_hbm.at[:, pl.ds(j * 128, 128)], v_v.at[j], sem_s.at[j]),
                 pltpu.make_async_copy(ssmk_hbm.at[pl.ds(j * 128, 128), :], ssmk_v.at[j], sem_s.at[j])]
                for j in range(NSLAB)]
    f_cps = [pltpu.make_async_copy(shift_hbm, shift_v, sem_f.at[0]),
             pltpu.make_async_copy(ssmd_hbm, ssmd_v, sem_f.at[0]),
             pltpu.make_async_copy(seed_hbm, seed_v, sem_f.at[0])]
    XA = 4 * SEG
    xa_cps = [pltpu.make_async_copy(x_hbm.at[pl.ds(0, XA), :], x_v.at[pl.ds(0, XA), :], sem_x.at[0]),
              pltpu.make_async_copy(mem0_hbm, mem0_v, sem_x.at[0])]
    xb_cp = pltpu.make_async_copy(x_hbm.at[pl.ds(XA, S_LEN - XA), :], x_v.at[pl.ds(XA, S_LEN - XA), :],
                                  sem_x.at[1])
    w_cps = []
    for m, w_hbm in enumerate((wq_hbm, wk_hbm, wv_hbm)):
        w32 = w_hbm.bitcast(U32)
        for j in range(32):
            w_cps.append(pltpu.make_async_copy(w32.at[:, j, :], wbuf.at[m * 32 + j], sem_w.at[0]))
    wo32 = wo_hbm.bitcast(U32)
    WO_SPLIT = (0, 24, 32)
    wo_cps = [pltpu.make_async_copy(wo32.at[pl.ds(a * 64, (b - a) * 64), :], wo_v.at[pl.ds(a * 64, (b - a) * 64), :],
                                    sem_wo.at[ci])
              for ci, (a, b) in enumerate(zip(WO_SPLIT[:-1], WO_SPLIT[1:]))]
    W_B0, W_B1 = 6, 30

    for c in f_cps + slab_cps[0]:
        c.start()

    r_i = lax.broadcasted_iota(jnp.int32, (ROWS, 128), 0)
    c_i = lax.broadcasted_iota(jnp.int32, (ROWS, 128), 1)
    same = jnp.logical_and((r_i < 40) == (c_i < 40), c_i < ROWS)
    memr = jnp.logical_and(r_i >= 32, r_i < 48)
    memc = jnp.logical_and(c_i >= 32, c_i < 48)
    ok = jnp.logical_or(jnp.logical_or(memr, memc), c_i <= r_i)
    log2e = float(np.log2(np.e))
    bias_s[...] = jnp.where(same, jnp.where(ok, np.float32(0.0), np.float32(-1e9 * log2e)),
                            np.float32(-1e30))
    r_l = lax.broadcasted_iota(jnp.int32, (48, 128), 0) + 32
    c_l = lax.broadcasted_iota(jnp.int32, (48, 128), 1) + 32
    same_l = jnp.logical_and((r_l < 40) == (c_l < 40), c_l < ROWS)
    ok_l = jnp.logical_or(jnp.logical_or(r_l < 48, c_l < 48), c_l <= r_l)
    biasl_s[...] = jnp.where(same_l, jnp.where(ok_l, np.float32(0.0), np.float32(-1e9 * log2e)),
                             np.float32(-1e30))
    kf_s[pl.ds(0, 8), :] = jnp.zeros((8, 128), F32)

    for c in f_cps:
        c.wait()
    for c in slab_cps[1]:
        c.start()
    ri0 = (lax.broadcasted_iota(jnp.int32, (64, 128), 1) // 8) % 2 == 0
    ffw_s[0] = pltpu.bitcast(seed_v[pl.ds(392, 128), :].astype(BF16), U32)
    fiv_s[0] = pltpu.bitcast(seed_v[pl.ds(520, 128), :].astype(BF16), U32)
    cdf, sdf = seed_v[pl.ds(384, 1), :], seed_v[pl.ds(385, 1), :]

    def gen_fwd(sl, cs):
        c0, s0 = cs
        c1 = c0 * cdf - s0 * sdf
        s1 = s0 * cdf + c0 * sdf
        top = jnp.where(ri0, c1, -s1)
        bot = jnp.where(ri0, s1, c1)
        ffw_s[sl] = pltpu.bitcast(jnp.concatenate([top, bot], axis=0).astype(BF16), U32)
        return c1, s1

    lax.fori_loop(1, 32, gen_fwd, (seed_v[pl.ds(0, 64), :], seed_v[pl.ds(64, 64), :]))

    def gen_inv(sl, cs):
        c0, s0 = cs
        cd, sd = seed_v[pl.ds(256, 64), :], seed_v[pl.ds(320, 64), :]
        c1 = c0 * cd - s0 * sd
        s1 = s0 * cd + c0 * sd
        top = jnp.where(ri0, c1, -s1)
        bot = jnp.where(ri0, s1, c1)
        fiv_s[sl] = pltpu.bitcast(jnp.concatenate([top, bot], axis=0).astype(BF16), U32)
        return c1, s1

    lax.fori_loop(1, 32, gen_inv, (seed_v[pl.ds(128, 64), :], seed_v[pl.ds(192, 64), :]))

    for c in slab_cps[0] + slab_cps[1]:
        c.wait()
    for c in slab_cps[2] + slab_cps[3] + slab_cps[4] + xa_cps + w_cps[:W_B0]:
        c.start()
    wrow_s[pl.ds(0, 4), :] = shift_v[...].astype(F32)
    wrow_s[pl.ds(4, 1), :] = ssmd_v[...].astype(F32).reshape(1, DM)
    row0 = lax.broadcasted_iota(jnp.int32, (8, 128), 0) == 0
    RB = 128

    def taps(j):
        lane0 = j * 128
        return ([wrow_s[pl.ds(t, 1), pl.ds(lane0, 128)] for t in range(4)],
                wrow_s[pl.ds(4, 1), pl.ds(lane0, 128)])

    def prep_p(j, r, n):
        kf_s[pl.ds(8 + r, n), :] = k_v[j, pl.ds(r, n), :].astype(F32)

    def prep_q(j, r, w):
        ks = (kf_s[pl.ds(8 + r, RB), :] * w[0] + kf_s[pl.ds(7 + r, RB), :] * w[1]
              + kf_s[pl.ds(6 + r, RB), :] * w[2] + kf_s[pl.ds(5 + r, RB), :] * w[3])
        kv_s[pl.ds(r, RB), :] = ks * v_v[j, pl.ds(r, RB), :].astype(F32)

    def prep_t(j, dd):
        ht = ssmk_v[j].astype(F32).T
        ht_s[pl.ds(8, S_LEN - 8), :] = ht[8:]
        ht_s[pl.ds(0, 8), :] = ht[:8] + jnp.where(row0, dd, np.float32(0.0))

    def pk(re, im):
        return jnp.concatenate([re, im], axis=0).astype(BF16)

    def fwd_nets(src, dst):
        def fwd_a(g, c):
            r = pl.multiple_of(g * 8, 8)
            r2 = pl.multiple_of(g * 16, 16)
            xs = [_SV(src[pl.ds(n2 * 64 + r, 8), :]) for n2 in range(32)]
            orr, oi = _odft(xs)
            for q in range(16):
                dst[2 * q + 1, pl.ds(r2, 16), :] = pk(orr[q].get(), oi[q].get())
            return c

        def fwd_b(g, c):
            r = pl.multiple_of(g * 8, 8)
            r2 = pl.multiple_of(g * 16, 16)
            xs = [_SV(src[pl.ds(n2 * 64 + r, 8), :]) for n2 in range(32)]
            er, ei = _rdft(xs)
            dst[0, pl.ds(r2, 16), :] = pk(er[0].get(), er[16].get())
            for q in range(1, 16):
                dst[2 * q, pl.ds(r2, 16), :] = pk(er[q].get(), ei[q].get())
            return c

        lax.fori_loop(0, 8, fwd_a, 0)
        lax.fori_loop(0, 8, fwd_b, 0)

    def inv_a(br, r):
        sr = [_SV(br[2 * q + 1, pl.ds(r, 8), :]) for q in range(16)]
        si = [_SV(br[2 * q + 1, pl.ds(64 + r, 8), :]) for q in range(16)]
        bb = _odft_T(sr, si)
        for n2 in range(32):
            ta_s[pl.ds(n2 * 64 + r, 8), :] = bb[n2].get()

    def inv_b(br, jy, r):
        sr = [None] * 17
        si = [None] * 17
        sr[0] = _SV(br[0, pl.ds(r, 8), :])
        sr[16] = _SV(br[0, pl.ds(64 + r, 8), :])
        for q in range(1, 16):
            sr[q] = _SV(br[2 * q, pl.ds(r, 8), :])
            si[q] = _SV(br[2 * q, pl.ds(64 + r, 8), :])
        aa = _rdft_T(sr, si)
        for n2 in range(32):
            prev = _SV(ta_s[pl.ds(n2 * 64 + r, 8), :])
            y_v[jy, pl.ds(n2 * 64 + r, 8), :] = (aa[n2] + prev).get()

    def mxu_block(j, bw, br):
        jn = j + 1
        jy = j - 1
        do_prep = j + 1 < NSLAB
        do_inv = j >= 1
        w, dd = taps(min(jn, NSLAB - 1))
        LAG = 3
        X, Y = {}, {}
        for t in range(32 + LAG):
            if do_prep and t % 8 == 0 and t < 32:
                nb = t // 2
                ht_s[pl.ds(nb * 128, 512), :] = ssmk_v[jn, :, pl.ds(nb * 128, 512)].astype(F32).T
            if do_prep and t % 2 == 0 and t < 32:
                prep_p(jn, (t // 2) * RB, RB)
            if do_prep and t % 2 == 1 and t < 32:
                prep_q(jn, (t // 2) * RB, w)
            if do_inv and t % 4 == 0 and t < 32:
                inv_a(br, (t // 4) * 8)
            if do_inv and t % 4 == 2 and t < 32:
                inv_b(br, jy, (t // 4) * 8)
            if t < 32:
                f = pltpu.bitcast(ffw_s[t], BF16)
                X[t] = (_mm(f, akv_s[t]), _mm(f, ah_s[t]))
            if 1 <= t <= 32:
                sl = t - 1
                xk, xh = X.pop(sl)
                kr, ki, hr, hi = xk[:64], xk[64:], xh[:64], xh[64:]
                yr = kr * hr - ki * hi
                yi = kr * hi + ki * hr
                if sl == 0:
                    yr = jnp.concatenate([jnp.where(row0, kr[:8] * hr[:8], yr[:8]), yr[8:]], axis=0)
                    yi = jnp.concatenate([jnp.where(row0, ki[:8] * hi[:8], yi[:8]), yi[8:]], axis=0)
                parts = []
                for jj in range(8):
                    parts.append(yr[8 * jj:8 * jj + 8])
                    parts.append(yi[8 * jj:8 * jj + 8])
                Y[sl] = jnp.concatenate(parts, axis=0).astype(BF16)
            if t >= LAG:
                sl = t - LAG
                bw[sl] = _mm(pltpu.bitcast(fiv_s[sl], BF16), Y.pop(sl))
        if do_prep:
            ht_s[pl.ds(0, 8), :] = ht_s[pl.ds(0, 8), :] + jnp.where(row0, dd, np.float32(0.0))

    w0, dd0 = taps(0)

    def p_body(b, c):
        prep_p(0, pl.multiple_of(b * 256, 256), 256)
        return c

    lax.fori_loop(0, S_LEN // 256, p_body, 0)

    def q_body(b, c):
        prep_q(0, pl.multiple_of(b * RB, RB), w0)
        return c

    lax.fori_loop(0, S_LEN // RB, q_body, 0)
    prep_t(0, dd0)

    for j in range(NSLAB):
        fwd_nets(kv_s, akv_s)
        fwd_nets(ht_s, ah_s)
        if j == 1:
            for c in slab_cps[2] + slab_cps[3] + slab_cps[4] + xa_cps:
                c.wait()
            for c in w_cps[W_B0:W_B1]:
                c.start()
        if j == 2:
            for c in w_cps[W_B1:] + wo_cps:
                c.start()
        mxu_block(j, (ba_s, bb_s)[j % 2], (ba_s, bb_s)[1 - j % 2])
    jl = NSLAB - 1

    def ia_body(g, c):
        inv_a(ba_s if jl % 2 == 0 else bb_s, pl.multiple_of(g * 8, 8))
        return c

    def ib_body(g, c):
        inv_b(ba_s if jl % 2 == 0 else bb_s, jl, pl.multiple_of(g * 8, 8))
        return c

    lax.fori_loop(0, 8, ia_body, 0)
    lax.fori_loop(0, 8, ib_body, 0)

    for c in w_cps:
        c.wait()

    def relayout_pair(p):
        for m in range(3):
            ia = m * 32 + p
            ib = ia + 16
            for r in range(0, 320, 64):
                a = wbuf[ia, pl.ds(r, 64), :]
                b = wbuf[ib, pl.ds(r, 64), :]
                wbuf[ia, pl.ds(r, 64), :] = (a & np.uint32(0xFFFF)) | (b << 16)
                wbuf[ib, pl.ds(r, 64), :] = (a >> 16) | (b & np.uint32(0xFFFF0000))

    def widx(m, h):
        return m * 32 + (h % 2) * 16 + h // 2

    LAGS_MID = (3, 10, 2)
    LAGS_EDGE = (4, 7, 6)
    cscale = np.float32(DH ** -0.5 * log2e)

    def load_y(idx):
        r0 = pl.multiple_of(idx * SEG, SEG)
        return jnp.concatenate([y_v[jj, pl.ds(r0, SEG), :] for jj in range(NSLAB)], axis=1)

    def wt(m, h):
        return pltpu.bitcast(wbuf[widx(m, h)], BF16)

    def filler(seg):
        rn = pl.multiple_of(seg * SEG, SEG)
        tok1 = _ln(x_v[pl.ds(rn, SEG), :].astype(F32)).astype(BF16)
        for h in range(NF):
            for m in range(3):
                q1_s[h * 3 + m] = _mm(tok1, wt(m, h)).astype(BF16)
        h_s[pl.ds(0, 32), :] = tok1

    def attention(kind):
        r0, r1 = {"first": (0, 48), "mid": (0, 80), "last": (32, 80)}[kind]
        R = r1 - r0
        H = h_s[pl.ds(r0, R), :]
        if kind == "last":
            HQ = h_s[pl.ds(48, 32), :]
            bias = biasl_s[pl.ds(16, 32), :]
        else:
            HQ = H
            bias = bias_s[pl.ds(0, R), :]
        valid = bias > np.float32(-1.0)
        bounds = (0, 8, 16, 24, 32)
        nf = NF if kind == "mid" else 0
        if nf:
            HB = h_s[pl.ds(32, 48), :]
        qkv, P, L, O = {}, {}, {}, {}
        acc = [None] * NSLAB
        zpad = jnp.zeros((128 - R, DH), BF16)

        def do_qkv(h):
            if h < nf:
                qkv[h] = tuple(jnp.concatenate([q1_s[h * 3 + m], _mm(HB, wt(m, h)).astype(BF16)], axis=0)
                               for m in range(3))
            else:
                qkv[h] = tuple(_mm(HQ if m == 0 else H, wt(m, h)).astype(BF16) for m in range(3))

        def do_s(h):
            q, k, v = qkv[h]
            sc = _mm_nt(q, jnp.concatenate([k, zpad], axis=0))
            t = jnp.where(valid, sc * cscale, bias)
            mx = jnp.max(t, axis=-1, keepdims=True)
            e = jnp.exp2(t - mx)
            L[h] = jnp.sum(e, axis=-1, keepdims=True)
            P[h] = e.astype(BF16)

        def do_pv(h):
            v = qkv[h][2]
            o = _mm(P[h], jnp.concatenate([v, zpad], axis=0))
            O[h] = (o * _recip(L[h])).astype(BF16)

        def do_wo(g):
            if kind == "first":
                for ci in range(len(wo_cps)):
                    if WO_SPLIT[ci] == bounds[g]:
                        wo_cps[ci].wait()
                        if ci + 1 == len(wo_cps):
                            xb_cp.start()
            og = jnp.concatenate([O[h] for h in range(bounds[g], bounds[g + 1])], axis=1)
            for n in range(NSLAB):
                wo_n = pltpu.bitcast(wo_v[pl.ds(bounds[g] * 64, (bounds[g + 1] - bounds[g]) * 64),
                                          pl.ds(n * 128, 128)], BF16)
                r = _mm(og, wo_n)
                acc[n] = r if acc[n] is None else acc[n] + r

        NG = len(bounds) - 1
        done_wo = 0
        LAG_S, LAG_PV, LAG_WO = LAGS_MID if kind == "mid" else LAGS_EDGE
        if kind == "first":
            LAG_WO = 2 * NH
        for h in range(NH + LAG_PV + 1):
            if kind == "first" and h % 2 == 0:
                if h == 0:
                    relayout_pair(0)
                if h + 2 < NH:
                    relayout_pair(h // 2 + 1)
            if h < NH:
                do_qkv(h)
            if LAG_S <= h < NH + LAG_S:
                do_s(h - LAG_S)
            if LAG_PV <= h < NH + LAG_PV:
                do_pv(h - LAG_PV)
            while done_wo < NG and bounds[done_wo + 1] - 1 + LAG_PV + LAG_WO <= h:
                do_wo(done_wo)
                done_wo += 1
        while done_wo < NG:
            do_wo(done_wo)
            done_wo += 1
        return acc

    def l2_epilogue(a2, seg):
        x2 = _rb(x1p_s[...] + _rb(a2))
        res = x2 + _rb(_rb(_ln(x2)) * load_y(seg))
        r = pl.multiple_of(seg * SEG, SEG)
        out_v[pl.ds(r, SEG), :] = res.astype(BF16)

    def out_copy(seg):
        r = pl.multiple_of(seg * SEG, SEG)
        return pltpu.make_async_copy(out_v.at[pl.ds(r, SEG), :], out_hbm.at[pl.ds(r, SEG), :], sem_out.at[0])

    def l1_epilogue(a1, seg):
        r1 = pl.multiple_of(seg * SEG, SEG)
        x1 = _rb(x_v[pl.ds(r1, SEG), :].astype(F32) + _rb(a1))
        x1p = _rb(x1 + _rb(_rb(_ln(x1)) * load_y(seg)))
        x1p_s[...] = x1p
        h_s[pl.ds(48, 32), :] = _ln(x1p).astype(BF16)

    mem0 = mem0_v[...]
    h_s[pl.ds(0, 32), :] = _ln(x_v[pl.ds(0, SEG), :].astype(F32)).astype(BF16)
    h_s[pl.ds(32, 16), :] = jnp.concatenate([mem0, mem0], axis=0)
    acc = attention("first")
    filler(1)
    accf = jnp.concatenate(acc, axis=1)
    l1_epilogue(accf[0:32], 0)
    h_s[pl.ds(32, 16), :] = jnp.concatenate([accf[32:40].astype(BF16), mem0], axis=0)

    def mid_step(i):
        acc = attention("mid")
        filler(jnp.minimum(i + 1, NSEG - 1))
        accf = jnp.concatenate(acc, axis=1)
        l2_epilogue(accf[48:80], i - 1)
        l1_epilogue(accf[0:32], i)
        h_s[pl.ds(32, 16), :] = accf[32:48].astype(BF16)
        out_copy(i - 1).start()

    def step(i, carry):
        mid_step(i)

        @pl.when(i == 2)
        def _():
            xb_cp.wait()

        return carry

    lax.fori_loop(1, NSEG, step, 0)

    acc = attention("last")
    accf = jnp.concatenate(acc, axis=1)
    l2_epilogue(accf, NSEG - 1)
    out_copy(NSEG - 1).start()

    def wait_body(i, carry):
        out_copy(i).wait()
        return carry

    lax.fori_loop(0, NSEG, wait_body, 0)


@functools.partial(jax.jit, static_argnames=("A_seg_len",))
def pallas_interleave_layers__memory_aug_recurrent_mem_tr__ssm_conv_h3__prompt_kernel(
    A_x, A_mem0, A_Wq, A_Wk, A_Wv, A_Wo, A_seg_len, B_q, B_k, B_v, B_shift_k, B_ssm_k, B_ssm_D,
):
    del B_q
    assert A_seg_len == SEG
    x = A_x.reshape(S_LEN, DM)
    mem0 = A_mem0.reshape(MEM, DM)
    wq = A_Wq.reshape(DM // 2, 2 * NH, DH)
    wk = A_Wk.reshape(DM // 2, 2 * NH, DH)
    wv = A_Wv.reshape(DM // 2, 2 * NH, DH)
    wo = A_Wo.reshape(NH * DH, DM)
    k = B_k.reshape(S_LEN, DM)
    v = B_v.reshape(S_LEN, DM)
    seed = jnp.asarray(_SEED_TAB)
    any_spec = pl.BlockSpec(memory_space=pl.ANY)
    V = pltpu.VMEM
    DMA = pltpu.SemaphoreType.DMA
    scratch = [
        V((S_LEN, DM), BF16),
        V((MEM, DM), BF16),
        V((96, DM // 2, DH), U32),
        V((NH * DH // 2, DM), U32),
        V((NSLAB, S_LEN, 128), BF16),
        V((NSLAB, S_LEN, 128), BF16),
        V((4, DM), BF16),
        V((NSLAB, 128, S_LEN), BF16),
        V((DM,), BF16),
        V((648, 128), F32),
        V((32, 64, 128), U32),
        V((32, 64, 128), U32),
        V((8, DM), F32),
        V((8 + S_LEN, 128), F32),
        V((S_LEN, 128), F32),
        V((S_LEN, 128), F32),
        V((32, 128, 128), BF16),
        V((32, 128, 128), BF16),
        V((32, 128, 128), F32),
        V((32, 128, 128), F32),
        V((S_LEN, 128), F32),
        V((NSLAB, S_LEN, 128), F32),
        V((S_LEN, DM), BF16),
        V((ROWS, DM), BF16),
        V((3 * NF, SEG, DH), BF16),
        V((SEG, DM), F32),
        V((ROWS, 128), F32),
        V((48, 128), F32),
        DMA((1,)), DMA((NSLAB,)), DMA((2,)), DMA((1,)), DMA((2,)), DMA((1,)),
    ]
    out = pl.pallas_call(
        _kernel,
        out_shape=jax.ShapeDtypeStruct((S_LEN, DM), BF16),
        in_specs=[any_spec] * 12,
        out_specs=any_spec,
        scratch_shapes=scratch,
        compiler_params=pltpu.CompilerParams(vmem_limit_bytes=100 * 1024 * 1024),
    )(x, mem0, wq, wk, wv, wo, k, v, B_shift_k.T, B_ssm_k, B_ssm_D, seed)
    return out.reshape(1, S_LEN, DM)
```

```python
import functools

import numpy as np

import jax
import jax.numpy as jnp
from jax import lax
import jax.experimental.pallas as pl
import jax.experimental.pallas.tpu as pltpu

F32 = jnp.float32
BF16 = jnp.bfloat16
U32 = jnp.uint32

S_LEN = 2048
DM = 640
NH = 32
DH = 128
MEM = 8
SEG = 32
NSEG = S_LEN // SEG
ROWS = 2 * (MEM + SEG)
NSLAB = DM // 128
NF = 5

_NFFT = 2 * S_LEN


def _build_slot0_tables():
    c = np.arange(128)
    n1 = (c // 16) * 8 + (c % 8)
    ri = (c // 8) % 2
    f0 = np.zeros((128, 128), np.float64)
    g0 = np.zeros((128, 128), np.float64)
    for col in range(128):
        n = n1[col]
        if ri[col] == 0:
            for q in range(32):
                f0[q, col] = np.cos(2 * np.pi * n * q / 64)
                f0[64 + q, col] = (-1.0) ** n if q == 0 else -np.sin(2 * np.pi * n * q / 64)
        else:
            for q in range(32, 64):
                a = -2.0 * np.pi * n * (32 + 64 * (q - 32)) / _NFFT
                f0[q, col] = np.cos(a)
                f0[64 + q, col] = np.sin(a)
    for col in range(128):
        q, r = n1[col], ri[col]
        for n in range(64):
            if q < 32:
                if q == 0:
                    g0[n, col] = (1.0 if r == 0 else (-1.0) ** n) / _NFFT
                else:
                    a = 2 * np.pi * n * q / 64
                    g0[n, col] = 2.0 * (np.cos(a) if r == 0 else -np.sin(a)) / _NFFT
            else:
                a = 2.0 * np.pi * n * (32 + 64 * (q - 32)) / _NFFT
                g0[64 + n, col] = 2.0 * (np.cos(a) if r == 0 else -np.sin(a)) / _NFFT
    return f0, g0


_FWD0, _INV0 = _build_slot0_tables()


class _SV:
    __slots__ = ("x", "s")

    def __init__(self, x, s=1):
        self.x = x
        self.s = s

    def __neg__(self):
        return _SV(self.x, -self.s)

    def __add__(self, o):
        if o is None:
            return self
        if self.s == o.s:
            return _SV(self.x + o.x, self.s)
        if self.s > 0:
            return _SV(self.x - o.x, 1)
        return _SV(o.x - self.x, 1)

    def __sub__(self, o):
        if o is None:
            return self
        return self + (-o)

    def scale(self, c):
        return _SV(self.x * np.float32(c * self.s), 1)

    def get(self):
        return self.x if self.s > 0 else -self.x


def _cfft(re, im, n, sgn):
    if n == 1:
        return re, im
    er, ei = _cfft(re[0::2], im[0::2], n // 2, sgn)
    orr, oi = _cfft(re[1::2], im[1::2], n // 2, sgn)
    outr = [None] * n
    outi = [None] * n
    h = float(np.sqrt(0.5))
    for k in range(n // 2):
        a, b = orr[k], oi[k]
        if k == 0:
            tr, ti = a, b
        elif 4 * k == n:
            tr, ti = (-b, a) if sgn > 0 else (b, -a)
        elif 8 * k == n:
            if sgn < 0:
                tr, ti = (a + b).scale(h), (b - a).scale(h)
            else:
                tr, ti = (a - b).scale(h), (a + b).scale(h)
        elif 8 * k == 3 * n:
            if sgn < 0:
                tr, ti = (b - a).scale(h), (a + b).scale(-h)
            else:
                tr, ti = (a + b).scale(-h), (a - b).scale(h)
        else:
            ang = sgn * 2 * np.pi * k / n
            c, s = float(np.cos(ang)), float(np.sin(ang))
            tr = a.scale(c) - b.scale(s)
            ti = a.scale(s) + b.scale(c)
        outr[k] = er[k] + tr
        outi[k] = ei[k] + ti
        outr[k + n // 2] = er[k] - tr
        outi[k + n // 2] = ei[k] - ti
    return outr, outi


def _odft(u):
    n = len(u)
    if n == 1:
        return [u[0]], [None]
    h = n // 2
    cr, ci = [], []
    for m in range(h):
        a, b = u[m], u[m + h]
        if m == 0:
            cr.append(a)
            ci.append(-b)
        else:
            ang = -2 * np.pi * m / (2 * n)
            c, s = float(np.cos(ang)), float(np.sin(ang))
            if 8 * m == 2 * n:
                hh = float(np.sqrt(0.5))
                cr.append((a - b).scale(hh))
                ci.append((a + b).scale(-hh))
            else:
                cr.append(a.scale(c) + b.scale(s))
                ci.append(a.scale(s) - b.scale(c))
    Cr, Ci = _cfft(cr, ci, h, -1)
    outr = [None] * h
    outi = [None] * h
    for j in range(h):
        if j % 2 == 0:
            outr[j], outi[j] = Cr[j // 2], Ci[j // 2]
        else:
            l = (j - 1) // 2
            outr[j], outi[j] = Cr[h - 1 - l], -Ci[h - 1 - l]
    return outr, outi


def _rdft(x):
    n = len(x)
    if n == 1:
        return [x[0]], [None]
    h = n // 2
    er, ei = _rdft([x[i] + x[i + h] for i in range(h)])
    orr, oi = _odft([x[i] - x[i + h] for i in range(h)])
    outr = [None] * (h + 1)
    outi = [None] * (h + 1)
    for k in range(h + 1):
        if k % 2 == 0:
            outr[k], outi[k] = er[k // 2], ei[k // 2]
        else:
            outr[k], outi[k] = orr[k // 2], oi[k // 2]
    return outr, outi


def _odft_T(sr, si):
    h = len(sr)
    n = 2 * h
    Cr = [None] * h
    Ci = [None] * h
    for j in range(h):
        if j % 2 == 0:
            Cr[j // 2], Ci[j // 2] = sr[j], si[j]
        else:
            l = (j - 1) // 2
            Cr[h - 1 - l], Ci[h - 1 - l] = sr[j], -si[j]
    cr, ci = _cfft(Cr, Ci, h, +1)
    lo, hi = [], []
    for m in range(h):
        if m == 0:
            lo.append(cr[0])
            hi.append(-ci[0])
        else:
            ang = -2 * np.pi * m / (2 * n)
            c, s = float(np.cos(ang)), float(np.sin(ang))
            if 8 * m == 2 * n:
                hh = float(np.sqrt(0.5))
                lo.append((cr[m] - ci[m]).scale(hh))
                hi.append((cr[m] + ci[m]).scale(-hh))
            else:
                lo.append(cr[m].scale(c) + ci[m].scale(s))
                hi.append(cr[m].scale(s) - ci[m].scale(c))
    return lo + hi


def _rdft_T(sr, si):
    h = len(sr) - 1
    if h == 0:
        return [sr[0]]
    ev_r, ev_i = sr[0::2], si[0::2]
    od_r, od_i = sr[1::2], si[1::2]
    s = _rdft_T(ev_r, ev_i)
    if h == 1:
        d = [od_r[0]]
    else:
        d = _odft_T(od_r, od_i)
    return [s[i] + d[i] for i in range(h)] + [s[i] - d[i] for i in range(h)]


def _mm(a, b):
    return jnp.dot(a, b, preferred_element_type=F32)


def _mm_nt(a, b):
    return lax.dot_general(a, b, (((1,), (1,)), ((), ())), preferred_element_type=F32)


def _ln(x):
    m = jnp.mean(x, axis=-1, keepdims=True)
    d = x - m
    v = jnp.mean(d * d, axis=-1, keepdims=True)
    return d * lax.rsqrt(v + np.float32(1e-5))


def _rb(x):
    return x.astype(BF16).astype(F32)


def _recip(l):
    r = pl.reciprocal(l, approx=True)
    return r * (np.float32(2.0) - l * r)


def _build_seed_table():
    c = np.arange(128)
    n1 = (c // 16) * 8 + (c % 8)
    k = np.arange(64)
    tab = np.zeros((648, 128), np.float64)
    th = -2.0 * np.pi * (n1[None, :] * k[:, None]) / 64.0
    tab[0:64], tab[64:128] = np.cos(th), np.sin(th)
    th = 2.0 * np.pi * (k[:, None] * n1[None, :]) / 64.0
    tab[128:192], tab[192:256] = np.cos(th) * (2.0 / _NFFT), np.sin(th) * (2.0 / _NFFT)
    dl = 2.0 * np.pi * k / _NFFT
    tab[256:320], tab[320:384] = np.cos(dl)[:, None], np.sin(dl)[:, None]
    dl = -2.0 * np.pi * n1 / _NFFT
    tab[384], tab[385] = np.cos(dl), np.sin(dl)
    tab[392:520] = _FWD0
    tab[520:648] = _INV0
    return tab.astype(np.float32)


_SEED_TAB = _build_seed_table()


def _kernel(x_hbm, mem0_hbm, wq_hbm, wk_hbm, wv_hbm, wo_hbm, k_hbm, v_hbm, shift_hbm,
            ssmk_hbm, ssmd_hbm, seed_hbm,
            out_hbm,
            x_v, mem0_v, wbuf, wo_v, k_v, v_v, shift_v, ssmk_v, ssmd_v, seed_v, ffw_s, fiv_s, wrow_s,
            kf_s, kv_s, ht_s, akv_s, ah_s, ba_s, bb_s, ta_s, y_v, out_v, h_s, q1_s, x1p_s, bias_s, biasl_s,
            sem_f, sem_s, sem_x, sem_w, sem_wo, sem_out):
    slab_cps = [[pltpu.make_async_copy(k_hbm.at[:, pl.ds(j * 128, 128)], k_v.at[j], sem_s.at[j]),
                 pltpu.make_async_copy(v_hbm.at[:, pl.ds(j * 128, 128)], v_v.at[j], sem_s.at[j]),
                 pltpu.make_async_copy(ssmk_hbm.at[pl.ds(j * 128, 128), :], ssmk_v.at[j], sem_s.at[j])]
                for j in range(NSLAB)]
    f_cps = [pltpu.make_async_copy(shift_hbm, shift_v, sem_f.at[0]),
             pltpu.make_async_copy(ssmd_hbm, ssmd_v, sem_f.at[0]),
             pltpu.make_async_copy(seed_hbm, seed_v, sem_f.at[0])]
    XA = 4 * SEG
    xa_cps = [pltpu.make_async_copy(x_hbm.at[pl.ds(0, XA), :], x_v.at[pl.ds(0, XA), :], sem_x.at[0]),
              pltpu.make_async_copy(mem0_hbm, mem0_v, sem_x.at[0])]
    xb_cp = pltpu.make_async_copy(x_hbm.at[pl.ds(XA, S_LEN - XA), :], x_v.at[pl.ds(XA, S_LEN - XA), :],
                                  sem_x.at[1])
    w_cps = []
    for m, w_hbm in enumerate((wq_hbm, wk_hbm, wv_hbm)):
        w32 = w_hbm.bitcast(U32)
        for j in range(32):
            w_cps.append(pltpu.make_async_copy(w32.at[:, j, :], wbuf.at[m * 32 + j], sem_w.at[0]))
    wo32 = wo_hbm.bitcast(U32)
    WO_SPLIT = (0, 24, 32)
    wo_cps = [pltpu.make_async_copy(wo32.at[pl.ds(a * 64, (b - a) * 64), :], wo_v.at[pl.ds(a * 64, (b - a) * 64), :],
                                    sem_wo.at[ci])
              for ci, (a, b) in enumerate(zip(WO_SPLIT[:-1], WO_SPLIT[1:]))]
    W_B0, W_B1 = 18, 40

    for c in f_cps + slab_cps[0]:
        c.start()

    r_i = lax.broadcasted_iota(jnp.int32, (ROWS, 128), 0)
    c_i = lax.broadcasted_iota(jnp.int32, (ROWS, 128), 1)
    same = jnp.logical_and((r_i < 40) == (c_i < 40), c_i < ROWS)
    memr = jnp.logical_and(r_i >= 32, r_i < 48)
    memc = jnp.logical_and(c_i >= 32, c_i < 48)
    ok = jnp.logical_or(jnp.logical_or(memr, memc), c_i <= r_i)
    log2e = float(np.log2(np.e))
    bias_s[...] = jnp.where(same, jnp.where(ok, np.float32(0.0), np.float32(-1e9 * log2e)),
                            np.float32(-1e30))
    r_l = lax.broadcasted_iota(jnp.int32, (48, 128), 0) + 32
    c_l = lax.broadcasted_iota(jnp.int32, (48, 128), 1) + 32
    same_l = jnp.logical_and((r_l < 40) == (c_l < 40), c_l < ROWS)
    ok_l = jnp.logical_or(jnp.logical_or(r_l < 48, c_l < 48), c_l <= r_l)
    biasl_s[...] = jnp.where(same_l, jnp.where(ok_l, np.float32(0.0), np.float32(-1e9 * log2e)),
                             np.float32(-1e30))
    kf_s[pl.ds(0, 8), :] = jnp.zeros((8, 128), F32)

    for c in f_cps:
        c.wait()
    for c in slab_cps[1]:
        c.start()
    ri0 = (lax.broadcasted_iota(jnp.int32, (64, 128), 1) // 8) % 2 == 0
    ffw_s[0] = pltpu.bitcast(seed_v[pl.ds(392, 128), :].astype(BF16), U32)
    fiv_s[0] = pltpu.bitcast(seed_v[pl.ds(520, 128), :].astype(BF16), U32)
    cdf, sdf = seed_v[pl.ds(384, 1), :], seed_v[pl.ds(385, 1), :]

    def gen_fwd(sl, cs):
        c0, s0 = cs
        c1 = c0 * cdf - s0 * sdf
        s1 = s0 * cdf + c0 * sdf
        top = jnp.where(ri0, c1, -s1)
        bot = jnp.where(ri0, s1, c1)
        ffw_s[sl] = pltpu.bitcast(jnp.concatenate([top, bot], axis=0).astype(BF16), U32)
        return c1, s1

    lax.fori_loop(1, 32, gen_fwd, (seed_v[pl.ds(0, 64), :], seed_v[pl.ds(64, 64), :]))

    def gen_inv(sl, cs):
        c0, s0 = cs
        cd, sd = seed_v[pl.ds(256, 64), :], seed_v[pl.ds(320, 64), :]
        c1 = c0 * cd - s0 * sd
        s1 = s0 * cd + c0 * sd
        top = jnp.where(ri0, c1, -s1)
        bot = jnp.where(ri0, s1, c1)
        fiv_s[sl] = pltpu.bitcast(jnp.concatenate([top, bot], axis=0).astype(BF16), U32)
        return c1, s1

    lax.fori_loop(1, 32, gen_inv, (seed_v[pl.ds(128, 64), :], seed_v[pl.ds(192, 64), :]))

    for c in slab_cps[2]:
        c.start()
    for c in slab_cps[0] + slab_cps[1]:
        c.wait()
    for c in slab_cps[3] + slab_cps[4] + xa_cps:
        c.start()
    wrow_s[pl.ds(0, 4), :] = shift_v[...].astype(F32)
    wrow_s[pl.ds(4, 1), :] = ssmd_v[...].astype(F32).reshape(1, DM)
    row0 = lax.broadcasted_iota(jnp.int32, (8, 128), 0) == 0
    RB = 128

    def taps(j):
        lane0 = j * 128
        return ([wrow_s[pl.ds(t, 1), pl.ds(lane0, 128)] for t in range(4)],
                wrow_s[pl.ds(4, 1), pl.ds(lane0, 128)])

    def prep_p(j, r, n):
        kf_s[pl.ds(8 + r, n), :] = k_v[j, pl.ds(r, n), :].astype(F32)

    def prep_q(j, r, w):
        ks = (kf_s[pl.ds(8 + r, RB), :] * w[0] + kf_s[pl.ds(7 + r, RB), :] * w[1]
              + kf_s[pl.ds(6 + r, RB), :] * w[2] + kf_s[pl.ds(5 + r, RB), :] * w[3])
        kv_s[pl.ds(r, RB), :] = ks * v_v[j, pl.ds(r, RB), :].astype(F32)

    def prep_t(j, dd):
        ht = ssmk_v[j].astype(F32).T
        ht_s[pl.ds(8, S_LEN - 8), :] = ht[8:]
        ht_s[pl.ds(0, 8), :] = ht[:8] + jnp.where(row0, dd, np.float32(0.0))

    def pk(re, im):
        return jnp.concatenate([re, im], axis=0).astype(BF16)

    def fwd_nets(src, dst):
        def fwd_a(g, c):
            r = pl.multiple_of(g * 8, 8)
            r2 = pl.multiple_of(g * 16, 16)
            xs = [_SV(src[pl.ds(n2 * 64 + r, 8), :]) for n2 in range(32)]
            orr, oi = _odft(xs)
            for q in range(16):
                dst[2 * q + 1, pl.ds(r2, 16), :] = pk(orr[q].get(), oi[q].get())
            return c

        def fwd_b(g, c):
            r = pl.multiple_of(g * 8, 8)
            r2 = pl.multiple_of(g * 16, 16)
            xs = [_SV(src[pl.ds(n2 * 64 + r, 8), :]) for n2 in range(32)]
            er, ei = _rdft(xs)
            dst[0, pl.ds(r2, 16), :] = pk(er[0].get(), er[16].get())
            for q in range(1, 16):
                dst[2 * q, pl.ds(r2, 16), :] = pk(er[q].get(), ei[q].get())
            return c

        lax.fori_loop(0, 8, fwd_a, 0)
        lax.fori_loop(0, 8, fwd_b, 0)

    def inv_a(br, r):
        sr = [_SV(br[2 * q + 1, pl.ds(r, 8), :]) for q in range(16)]
        si = [_SV(br[2 * q + 1, pl.ds(64 + r, 8), :]) for q in range(16)]
        bb = _odft_T(sr, si)
        for n2 in range(32):
            ta_s[pl.ds(n2 * 64 + r, 8), :] = bb[n2].get()

    def inv_b(br, jy, r):
        sr = [None] * 17
        si = [None] * 17
        sr[0] = _SV(br[0, pl.ds(r, 8), :])
        sr[16] = _SV(br[0, pl.ds(64 + r, 8), :])
        for q in range(1, 16):
            sr[q] = _SV(br[2 * q, pl.ds(r, 8), :])
            si[q] = _SV(br[2 * q, pl.ds(64 + r, 8), :])
        aa = _rdft_T(sr, si)
        for n2 in range(32):
            prev = _SV(ta_s[pl.ds(n2 * 64 + r, 8), :])
            y_v[jy, pl.ds(n2 * 64 + r, 8), :] = (aa[n2] + prev).get()

    def mxu_block(j, bw, br):
        jn = j + 1
        jy = j - 1
        do_prep = j + 1 < NSLAB
        do_inv = j >= 1
        w, dd = taps(min(jn, NSLAB - 1))
        LAG = 3
        X, Y = {}, {}
        for t in range(32 + LAG):
            if do_prep and t % 8 == 0 and t < 32:
                nb = t // 2
                ht_s[pl.ds(nb * 128, 512), :] = ssmk_v[jn, :, pl.ds(nb * 128, 512)].astype(F32).T
            if do_prep and t % 2 == 0 and t < 32:
                prep_p(jn, (t // 2) * RB, RB)
            if do_prep and t % 2 == 1 and t < 32:
                prep_q(jn, (t // 2) * RB, w)
            if do_inv and t % 4 == 0 and t < 32:
                inv_a(br, (t // 4) * 8)
            if do_inv and t % 4 == 2 and t < 32:
                inv_b(br, jy, (t // 4) * 8)
            if t < 32:
                f = pltpu.bitcast(ffw_s[t], BF16)
                X[t] = (_mm(f, akv_s[t]), _mm(f, ah_s[t]))
            if 1 <= t <= 32:
                sl = t - 1
                xk, xh = X.pop(sl)
                kr, ki, hr, hi = xk[:64], xk[64:], xh[:64], xh[64:]
                yr = kr * hr - ki * hi
                yi = kr * hi + ki * hr
                if sl == 0:
                    yr = jnp.concatenate([jnp.where(row0, kr[:8] * hr[:8], yr[:8]), yr[8:]], axis=0)
                    yi = jnp.concatenate([jnp.where(row0, ki[:8] * hi[:8], yi[:8]), yi[8:]], axis=0)
                parts = []
                for jj in range(8):
                    parts.append(yr[8 * jj:8 * jj + 8])
                    parts.append(yi[8 * jj:8 * jj + 8])
                Y[sl] = jnp.concatenate(parts, axis=0).astype(BF16)
            if t >= LAG:
                sl = t - LAG
                bw[sl] = _mm(pltpu.bitcast(fiv_s[sl], BF16), Y.pop(sl))
        if do_prep:
            ht_s[pl.ds(0, 8), :] = ht_s[pl.ds(0, 8), :] + jnp.where(row0, dd, np.float32(0.0))

    w0, dd0 = taps(0)

    def p_body(b, c):
        prep_p(0, pl.multiple_of(b * 256, 256), 256)
        return c

    lax.fori_loop(0, S_LEN // 256, p_body, 0)

    def q_body(b, c):
        prep_q(0, pl.multiple_of(b * RB, RB), w0)
        return c

    lax.fori_loop(0, S_LEN // RB, q_body, 0)
    prep_t(0, dd0)

    for j in range(NSLAB):
        if j == 1:
            for c in w_cps[:W_B0]:
                c.start()
        fwd_nets(kv_s, akv_s)
        fwd_nets(ht_s, ah_s)
        if j == 1:
            for c in slab_cps[2] + slab_cps[3] + slab_cps[4] + xa_cps:
                c.wait()
            for c in w_cps[W_B0:W_B1]:
                c.start()
        if j == 2:
            for c in w_cps[W_B1:] + wo_cps:
                c.start()
        mxu_block(j, (ba_s, bb_s)[j % 2], (ba_s, bb_s)[1 - j % 2])
    jl = NSLAB - 1

    def ia_body(g, c):
        inv_a(ba_s if jl % 2 == 0 else bb_s, pl.multiple_of(g * 8, 8))
        return c

    def ib_body(g, c):
        inv_b(ba_s if jl % 2 == 0 else bb_s, jl, pl.multiple_of(g * 8, 8))
        return c

    lax.fori_loop(0, 8, ia_body, 0)
    lax.fori_loop(0, 8, ib_body, 0)

    for c in w_cps:
        c.wait()

    def relayout_pair(p):
        for m in range(3):
            ia = m * 32 + p
            ib = ia + 16
            for r in range(0, 320, 64):
                a = wbuf[ia, pl.ds(r, 64), :]
                b = wbuf[ib, pl.ds(r, 64), :]
                wbuf[ia, pl.ds(r, 64), :] = (a & np.uint32(0xFFFF)) | (b << 16)
                wbuf[ib, pl.ds(r, 64), :] = (a >> 16) | (b & np.uint32(0xFFFF0000))

    def widx(m, h):
        return m * 32 + (h % 2) * 16 + h // 2

    LAGS_MID = (3, 10, 2)
    LAGS_EDGE = (4, 7, 6)
    cscale = np.float32(DH ** -0.5 * log2e)

    def load_y(idx):
        r0 = pl.multiple_of(idx * SEG, SEG)
        return jnp.concatenate([y_v[jj, pl.ds(r0, SEG), :] for jj in range(NSLAB)], axis=1)

    def wt(m, h):
        return pltpu.bitcast(wbuf[widx(m, h)], BF16)

    def filler(seg):
        rn = pl.multiple_of(seg * SEG, SEG)
        tok1 = _ln(x_v[pl.ds(rn, SEG), :].astype(F32)).astype(BF16)
        for h in range(NF):
            for m in range(3):
                q1_s[h * 3 + m] = _mm(tok1, wt(m, h)).astype(BF16)
        h_s[pl.ds(0, 32), :] = tok1

    def attention(kind):
        r0, r1 = {"first": (0, 48), "mid": (0, 80), "last": (32, 80)}[kind]
        R = r1 - r0
        H = h_s[pl.ds(r0, R), :]
        if kind == "last":
            HQ = h_s[pl.ds(48, 32), :]
            bias = biasl_s[pl.ds(16, 32), :]
        else:
            HQ = H
            bias = bias_s[pl.ds(0, R), :]
        valid = bias > np.float32(-1.0)
        bounds = (0, 8, 16, 24, 32)
        nf = NF if kind == "mid" else 0
        if nf:
            HB = h_s[pl.ds(32, 48), :]
        qkv, P, L, O = {}, {}, {}, {}
        acc = [None] * NSLAB
        zpad = jnp.zeros((128 - R, DH), BF16)

        def do_qkv(h):
            if h < nf:
                qkv[h] = tuple(jnp.concatenate([q1_s[h * 3 + m], _mm(HB, wt(m, h)).astype(BF16)], axis=0)
                               for m in range(3))
            else:
                qkv[h] = tuple(_mm(HQ if m == 0 else H, wt(m, h)).astype(BF16) for m in range(3))

        def do_s(h):
            q, k, v = qkv[h]
            sc = _mm_nt(q, jnp.concatenate([k, zpad], axis=0))
            t = jnp.where(valid, sc * cscale, bias)
            mx = jnp.max(t, axis=-1, keepdims=True)
            e = jnp.exp2(t - mx)
            L[h] = jnp.sum(e, axis=-1, keepdims=True)
            P[h] = e.astype(BF16)

        def do_pv(h):
            v = qkv[h][2]
            o = _mm(P[h], jnp.concatenate([v, zpad], axis=0))
            O[h] = (o * _recip(L[h])).astype(BF16)

        def do_wo(g):
            if kind == "first":
                for ci in range(len(wo_cps)):
                    if WO_SPLIT[ci] == bounds[g]:
                        wo_cps[ci].wait()
                        if ci + 1 == len(wo_cps):
                            xb_cp.start()
            og = jnp.concatenate([O[h] for h in range(bounds[g], bounds[g + 1])], axis=1)
            for n in range(NSLAB):
                wo_n = pltpu.bitcast(wo_v[pl.ds(bounds[g] * 64, (bounds[g + 1] - bounds[g]) * 64),
                                          pl.ds(n * 128, 128)], BF16)
                r = _mm(og, wo_n)
                acc[n] = r if acc[n] is None else acc[n] + r

        NG = len(bounds) - 1
        done_wo = 0
        LAG_S, LAG_PV, LAG_WO = LAGS_MID if kind == "mid" else LAGS_EDGE
        if kind == "first":
            LAG_WO = 2 * NH
        for h in range(NH + LAG_PV + 1):
            if kind == "first" and h % 2 == 0:
                if h == 0:
                    relayout_pair(0)
                if h + 2 < NH:
                    relayout_pair(h // 2 + 1)
            if h < NH:
                do_qkv(h)
            if LAG_S <= h < NH + LAG_S:
                do_s(h - LAG_S)
            if LAG_PV <= h < NH + LAG_PV:
                do_pv(h - LAG_PV)
            while done_wo < NG and bounds[done_wo + 1] - 1 + LAG_PV + LAG_WO <= h:
                do_wo(done_wo)
                done_wo += 1
        while done_wo < NG:
            do_wo(done_wo)
            done_wo += 1
        return acc

    def l2_epilogue(a2, seg):
        x2 = _rb(x1p_s[...] + _rb(a2))
        res = x2 + _rb(_rb(_ln(x2)) * load_y(seg))
        r = pl.multiple_of(seg * SEG, SEG)
        out_v[pl.ds(r, SEG), :] = res.astype(BF16)

    def out_copy(seg):
        r = pl.multiple_of(seg * SEG, SEG)
        return pltpu.make_async_copy(out_v.at[pl.ds(r, SEG), :], out_hbm.at[pl.ds(r, SEG), :], sem_out.at[0])

    def l1_epilogue(a1, seg):
        r1 = pl.multiple_of(seg * SEG, SEG)
        x1 = _rb(x_v[pl.ds(r1, SEG), :].astype(F32) + _rb(a1))
        x1p = _rb(x1 + _rb(_rb(_ln(x1)) * load_y(seg)))
        x1p_s[...] = x1p
        h_s[pl.ds(48, 32), :] = _ln(x1p).astype(BF16)

    mem0 = mem0_v[...]
    h_s[pl.ds(0, 32), :] = _ln(x_v[pl.ds(0, SEG), :].astype(F32)).astype(BF16)
    h_s[pl.ds(32, 16), :] = jnp.concatenate([mem0, mem0], axis=0)
    acc = attention("first")
    filler(1)
    accf = jnp.concatenate(acc, axis=1)
    l1_epilogue(accf[0:32], 0)
    h_s[pl.ds(32, 16), :] = jnp.concatenate([accf[32:40].astype(BF16), mem0], axis=0)

    def mid_step(i):
        acc = attention("mid")
        filler(jnp.minimum(i + 1, NSEG - 1))
        accf = jnp.concatenate(acc, axis=1)
        l2_epilogue(accf[48:80], i - 1)
        l1_epilogue(accf[0:32], i)
        h_s[pl.ds(32, 16), :] = accf[32:48].astype(BF16)
        out_copy(i - 1).start()

    def step(i, carry):
        mid_step(i)

        @pl.when(i == 2)
        def _():
            xb_cp.wait()

        return carry

    lax.fori_loop(1, NSEG, step, 0)

    acc = attention("last")
    accf = jnp.concatenate(acc, axis=1)
    l2_epilogue(accf, NSEG - 1)
    out_copy(NSEG - 1).start()

    def wait_body(i, carry):
        out_copy(i).wait()
        return carry

    lax.fori_loop(0, NSEG, wait_body, 0)


@functools.partial(jax.jit, static_argnames=("A_seg_len",))
def pallas_interleave_layers__memory_aug_recurrent_mem_tr__ssm_conv_h3__prompt_kernel(
    A_x, A_mem0, A_Wq, A_Wk, A_Wv, A_Wo, A_seg_len, B_q, B_k, B_v, B_shift_k, B_ssm_k, B_ssm_D,
):
    del B_q
    assert A_seg_len == SEG
    x = A_x.reshape(S_LEN, DM)
    mem0 = A_mem0.reshape(MEM, DM)
    wq = A_Wq.reshape(DM // 2, 2 * NH, DH)
    wk = A_Wk.reshape(DM // 2, 2 * NH, DH)
    wv = A_Wv.reshape(DM // 2, 2 * NH, DH)
    wo = A_Wo.reshape(NH * DH, DM)
    k = B_k.reshape(S_LEN, DM)
    v = B_v.reshape(S_LEN, DM)
    seed = jnp.asarray(_SEED_TAB)
    any_spec = pl.BlockSpec(memory_space=pl.ANY)
    V = pltpu.VMEM
    DMA = pltpu.SemaphoreType.DMA
    scratch = [
        V((S_LEN, DM), BF16),
        V((MEM, DM), BF16),
        V((96, DM // 2, DH), U32),
        V((NH * DH // 2, DM), U32),
        V((NSLAB, S_LEN, 128), BF16),
        V((NSLAB, S_LEN, 128), BF16),
        V((4, DM), BF16),
        V((NSLAB, 128, S_LEN), BF16),
        V((DM,), BF16),
        V((648, 128), F32),
        V((32, 64, 128), U32),
        V((32, 64, 128), U32),
        V((8, DM), F32),
        V((8 + S_LEN, 128), F32),
        V((S_LEN, 128), F32),
        V((S_LEN, 128), F32),
        V((32, 128, 128), BF16),
        V((32, 128, 128), BF16),
        V((32, 128, 128), F32),
        V((32, 128, 128), F32),
        V((S_LEN, 128), F32),
        V((NSLAB, S_LEN, 128), F32),
        V((S_LEN, DM), BF16),
        V((ROWS, DM), BF16),
        V((3 * NF, SEG, DH), BF16),
        V((SEG, DM), F32),
        V((ROWS, 128), F32),
        V((48, 128), F32),
        DMA((1,)), DMA((NSLAB,)), DMA((2,)), DMA((1,)), DMA((2,)), DMA((1,)),
    ]
    out = pl.pallas_call(
        _kernel,
        out_shape=jax.ShapeDtypeStruct((S_LEN, DM), BF16),
        in_specs=[any_spec] * 12,
        out_specs=any_spec,
        scratch_shapes=scratch,
        compiler_params=pltpu.CompilerParams(vmem_limit_bytes=100 * 1024 * 1024),
    )(x, mem0, wq, wk, wv, wo, k, v, B_shift_k.T, B_ssm_k, B_ssm_D, seed)
    return out.reshape(1, S_LEN, DM)
```

```python
import functools

import numpy as np

import jax
import jax.numpy as jnp
from jax import lax
import jax.experimental.pallas as pl
import jax.experimental.pallas.tpu as pltpu

F32 = jnp.float32
BF16 = jnp.bfloat16
U32 = jnp.uint32

S_LEN = 2048
DM = 640
NH = 32
DH = 128
MEM = 8
SEG = 32
NSEG = S_LEN // SEG
ROWS = 2 * (MEM + SEG)
NSLAB = DM // 128
NF = 5

_NFFT = 2 * S_LEN


def _build_slot0_tables():
    c = np.arange(128)
    n1 = (c // 16) * 8 + (c % 8)
    ri = (c // 8) % 2
    f0 = np.zeros((128, 128), np.float64)
    g0 = np.zeros((128, 128), np.float64)
    for col in range(128):
        n = n1[col]
        if ri[col] == 0:
            for q in range(32):
                f0[q, col] = np.cos(2 * np.pi * n * q / 64)
                f0[64 + q, col] = (-1.0) ** n if q == 0 else -np.sin(2 * np.pi * n * q / 64)
        else:
            for q in range(32, 64):
                a = -2.0 * np.pi * n * (32 + 64 * (q - 32)) / _NFFT
                f0[q, col] = np.cos(a)
                f0[64 + q, col] = np.sin(a)
    for col in range(128):
        q, r = n1[col], ri[col]
        for n in range(64):
            if q < 32:
                if q == 0:
                    g0[n, col] = (1.0 if r == 0 else (-1.0) ** n) / _NFFT
                else:
                    a = 2 * np.pi * n * q / 64
                    g0[n, col] = 2.0 * (np.cos(a) if r == 0 else -np.sin(a)) / _NFFT
            else:
                a = 2.0 * np.pi * n * (32 + 64 * (q - 32)) / _NFFT
                g0[64 + n, col] = 2.0 * (np.cos(a) if r == 0 else -np.sin(a)) / _NFFT
    return f0, g0


_FWD0, _INV0 = _build_slot0_tables()


class _SV:
    __slots__ = ("x", "s")

    def __init__(self, x, s=1):
        self.x = x
        self.s = s

    def __neg__(self):
        return _SV(self.x, -self.s)

    def __add__(self, o):
        if o is None:
            return self
        if self.s == o.s:
            return _SV(self.x + o.x, self.s)
        if self.s > 0:
            return _SV(self.x - o.x, 1)
        return _SV(o.x - self.x, 1)

    def __sub__(self, o):
        if o is None:
            return self
        return self + (-o)

    def scale(self, c):
        return _SV(self.x * np.float32(c * self.s), 1)

    def get(self):
        return self.x if self.s > 0 else -self.x


def _cfft(re, im, n, sgn):
    if n == 1:
        return re, im
    er, ei = _cfft(re[0::2], im[0::2], n // 2, sgn)
    orr, oi = _cfft(re[1::2], im[1::2], n // 2, sgn)
    outr = [None] * n
    outi = [None] * n
    h = float(np.sqrt(0.5))
    for k in range(n // 2):
        a, b = orr[k], oi[k]
        if k == 0:
            tr, ti = a, b
        elif 4 * k == n:
            tr, ti = (-b, a) if sgn > 0 else (b, -a)
        elif 8 * k == n:
            if sgn < 0:
                tr, ti = (a + b).scale(h), (b - a).scale(h)
            else:
                tr, ti = (a - b).scale(h), (a + b).scale(h)
        elif 8 * k == 3 * n:
            if sgn < 0:
                tr, ti = (b - a).scale(h), (a + b).scale(-h)
            else:
                tr, ti = (a + b).scale(-h), (a - b).scale(h)
        else:
            ang = sgn * 2 * np.pi * k / n
            c, s = float(np.cos(ang)), float(np.sin(ang))
            tr = a.scale(c) - b.scale(s)
            ti = a.scale(s) + b.scale(c)
        outr[k] = er[k] + tr
        outi[k] = ei[k] + ti
        outr[k + n // 2] = er[k] - tr
        outi[k + n // 2] = ei[k] - ti
    return outr, outi


def _odft(u):
    n = len(u)
    if n == 1:
        return [u[0]], [None]
    h = n // 2
    cr, ci = [], []
    for m in range(h):
        a, b = u[m], u[m + h]
        if m == 0:
            cr.append(a)
            ci.append(-b)
        else:
            ang = -2 * np.pi * m / (2 * n)
            c, s = float(np.cos(ang)), float(np.sin(ang))
            if 8 * m == 2 * n:
                hh = float(np.sqrt(0.5))
                cr.append((a - b).scale(hh))
                ci.append((a + b).scale(-hh))
            else:
                cr.append(a.scale(c) + b.scale(s))
                ci.append(a.scale(s) - b.scale(c))
    Cr, Ci = _cfft(cr, ci, h, -1)
    outr = [None] * h
    outi = [None] * h
    for j in range(h):
        if j % 2 == 0:
            outr[j], outi[j] = Cr[j // 2], Ci[j // 2]
        else:
            l = (j - 1) // 2
            outr[j], outi[j] = Cr[h - 1 - l], -Ci[h - 1 - l]
    return outr, outi


def _rdft(x):
    n = len(x)
    if n == 1:
        return [x[0]], [None]
    h = n // 2
    er, ei = _rdft([x[i] + x[i + h] for i in range(h)])
    orr, oi = _odft([x[i] - x[i + h] for i in range(h)])
    outr = [None] * (h + 1)
    outi = [None] * (h + 1)
    for k in range(h + 1):
        if k % 2 == 0:
            outr[k], outi[k] = er[k // 2], ei[k // 2]
        else:
            outr[k], outi[k] = orr[k // 2], oi[k // 2]
    return outr, outi


def _odft_T(sr, si):
    h = len(sr)
    n = 2 * h
    Cr = [None] * h
    Ci = [None] * h
    for j in range(h):
        if j % 2 == 0:
            Cr[j // 2], Ci[j // 2] = sr[j], si[j]
        else:
            l = (j - 1) // 2
            Cr[h - 1 - l], Ci[h - 1 - l] = sr[j], -si[j]
    cr, ci = _cfft(Cr, Ci, h, +1)
    lo, hi = [], []
    for m in range(h):
        if m == 0:
            lo.append(cr[0])
            hi.append(-ci[0])
        else:
            ang = -2 * np.pi * m / (2 * n)
            c, s = float(np.cos(ang)), float(np.sin(ang))
            if 8 * m == 2 * n:
                hh = float(np.sqrt(0.5))
                lo.append((cr[m] - ci[m]).scale(hh))
                hi.append((cr[m] + ci[m]).scale(-hh))
            else:
                lo.append(cr[m].scale(c) + ci[m].scale(s))
                hi.append(cr[m].scale(s) - ci[m].scale(c))
    return lo + hi


def _rdft_T(sr, si):
    h = len(sr) - 1
    if h == 0:
        return [sr[0]]
    ev_r, ev_i = sr[0::2], si[0::2]
    od_r, od_i = sr[1::2], si[1::2]
    s = _rdft_T(ev_r, ev_i)
    if h == 1:
        d = [od_r[0]]
    else:
        d = _odft_T(od_r, od_i)
    return [s[i] + d[i] for i in range(h)] + [s[i] - d[i] for i in range(h)]


def _mm(a, b):
    return jnp.dot(a, b, preferred_element_type=F32)


def _mm_nt(a, b):
    return lax.dot_general(a, b, (((1,), (1,)), ((), ())), preferred_element_type=F32)


def _ln(x):
    m = jnp.mean(x, axis=-1, keepdims=True)
    d = x - m
    v = jnp.mean(d * d, axis=-1, keepdims=True)
    return d * lax.rsqrt(v + np.float32(1e-5))


def _rb(x):
    return x.astype(BF16).astype(F32)


try:
    _reciprocal = pltpu.reciprocal
except AttributeError:
    _reciprocal = pl.reciprocal


def _recip(l):
    r = _reciprocal(l, approx=True)
    return r * (np.float32(2.0) - l * r)


def _build_seed_table():
    c = np.arange(128)
    n1 = (c // 16) * 8 + (c % 8)
    k = np.arange(64)
    tab = np.zeros((648, 128), np.float64)
    th = -2.0 * np.pi * (n1[None, :] * k[:, None]) / 64.0
    tab[0:64], tab[64:128] = np.cos(th), np.sin(th)
    th = 2.0 * np.pi * (k[:, None] * n1[None, :]) / 64.0
    tab[128:192], tab[192:256] = np.cos(th) * (2.0 / _NFFT), np.sin(th) * (2.0 / _NFFT)
    dl = 2.0 * np.pi * k / _NFFT
    tab[256:320], tab[320:384] = np.cos(dl)[:, None], np.sin(dl)[:, None]
    dl = -2.0 * np.pi * n1 / _NFFT
    tab[384], tab[385] = np.cos(dl), np.sin(dl)
    tab[392:520] = _FWD0
    tab[520:648] = _INV0
    return tab.astype(np.float32)


_SEED_TAB = _build_seed_table()


def _kernel(x_hbm, mem0_hbm, wq_hbm, wk_hbm, wv_hbm, wo_hbm, k_hbm, v_hbm, shift_hbm,
            ssmk_hbm, ssmd_hbm, seed_hbm,
            out_hbm,
            x_v, mem0_v, wbuf, wo_v, k_v, v_v, shift_v, ssmk_v, ssmd_v, seed_v, ffw_s, fiv_s, wrow_s,
            kf_s, kv_s, ht_s, akv_s, ah_s, ba_s, bb_s, ta_s, y_v, out_v, h_s, q1_s, x1p_s, bias_s, biasl_s,
            sem_f, sem_s, sem_x, sem_w, sem_wo, sem_out):
    slab_cps = [[pltpu.make_async_copy(k_hbm.at[:, pl.ds(j * 128, 128)], k_v.at[j], sem_s.at[j]),
                 pltpu.make_async_copy(v_hbm.at[:, pl.ds(j * 128, 128)], v_v.at[j], sem_s.at[j]),
                 pltpu.make_async_copy(ssmk_hbm.at[pl.ds(j * 128, 128), :], ssmk_v.at[j], sem_s.at[j])]
                for j in range(NSLAB)]
    f_cps = [pltpu.make_async_copy(shift_hbm, shift_v, sem_f.at[0]),
             pltpu.make_async_copy(ssmd_hbm, ssmd_v, sem_f.at[0]),
             pltpu.make_async_copy(seed_hbm, seed_v, sem_f.at[0])]
    XA = 4 * SEG
    xa_cps = [pltpu.make_async_copy(x_hbm.at[pl.ds(0, XA), :], x_v.at[pl.ds(0, XA), :], sem_x.at[0]),
              pltpu.make_async_copy(mem0_hbm, mem0_v, sem_x.at[0])]
    xb_cp = pltpu.make_async_copy(x_hbm.at[pl.ds(XA, S_LEN - XA), :], x_v.at[pl.ds(XA, S_LEN - XA), :],
                                  sem_x.at[1])
    w_cps = []
    for m, w_hbm in enumerate((wq_hbm, wk_hbm, wv_hbm)):
        w32 = w_hbm.bitcast(U32)
        for j in range(32):
            w_cps.append(pltpu.make_async_copy(w32.at[:, j, :], wbuf.at[m * 32 + j], sem_w.at[0]))
    wo32 = wo_hbm.bitcast(U32)
    WO_SPLIT = (0, 24, 32)
    wo_cps = [pltpu.make_async_copy(wo32.at[pl.ds(a * 64, (b - a) * 64), :], wo_v.at[pl.ds(a * 64, (b - a) * 64), :],
                                    sem_wo.at[ci])
              for ci, (a, b) in enumerate(zip(WO_SPLIT[:-1], WO_SPLIT[1:]))]
    W_B0, W_B1 = 18, 40

    for c in f_cps + slab_cps[0]:
        c.start()

    r_i = lax.broadcasted_iota(jnp.int32, (ROWS, 128), 0)
    c_i = lax.broadcasted_iota(jnp.int32, (ROWS, 128), 1)
    same = jnp.logical_and((r_i < 40) == (c_i < 40), c_i < ROWS)
    memr = jnp.logical_and(r_i >= 32, r_i < 48)
    memc = jnp.logical_and(c_i >= 32, c_i < 48)
    ok = jnp.logical_or(jnp.logical_or(memr, memc), c_i <= r_i)
    log2e = float(np.log2(np.e))
    bias_s[...] = jnp.where(same, jnp.where(ok, np.float32(0.0), np.float32(-1e9 * log2e)),
                            np.float32(-1e30))
    r_l = lax.broadcasted_iota(jnp.int32, (48, 128), 0) + 32
    c_l = lax.broadcasted_iota(jnp.int32, (48, 128), 1) + 32
    same_l = jnp.logical_and((r_l < 40) == (c_l < 40), c_l < ROWS)
    ok_l = jnp.logical_or(jnp.logical_or(r_l < 48, c_l < 48), c_l <= r_l)
    biasl_s[...] = jnp.where(same_l, jnp.where(ok_l, np.float32(0.0), np.float32(-1e9 * log2e)),
                             np.float32(-1e30))
    kf_s[pl.ds(0, 8), :] = jnp.zeros((8, 128), F32)

    for c in f_cps:
        c.wait()
    for c in slab_cps[1]:
        c.start()
    ri0 = (lax.broadcasted_iota(jnp.int32, (64, 128), 1) // 8) % 2 == 0
    ffw_s[0] = pltpu.bitcast(seed_v[pl.ds(392, 128), :].astype(BF16), U32)
    fiv_s[0] = pltpu.bitcast(seed_v[pl.ds(520, 128), :].astype(BF16), U32)
    cdf, sdf = seed_v[pl.ds(384, 1), :], seed_v[pl.ds(385, 1), :]

    def gen_fwd(sl, cs):
        c0, s0 = cs
        c1 = c0 * cdf - s0 * sdf
        s1 = s0 * cdf + c0 * sdf
        top = jnp.where(ri0, c1, -s1)
        bot = jnp.where(ri0, s1, c1)
        ffw_s[sl] = pltpu.bitcast(jnp.concatenate([top, bot], axis=0).astype(BF16), U32)
        return c1, s1

    lax.fori_loop(1, 32, gen_fwd, (seed_v[pl.ds(0, 64), :], seed_v[pl.ds(64, 64), :]))

    def gen_inv(sl, cs):
        c0, s0 = cs
        cd, sd = seed_v[pl.ds(256, 64), :], seed_v[pl.ds(320, 64), :]
        c1 = c0 * cd - s0 * sd
        s1 = s0 * cd + c0 * sd
        top = jnp.where(ri0, c1, -s1)
        bot = jnp.where(ri0, s1, c1)
        fiv_s[sl] = pltpu.bitcast(jnp.concatenate([top, bot], axis=0).astype(BF16), U32)
        return c1, s1

    lax.fori_loop(1, 32, gen_inv, (seed_v[pl.ds(128, 64), :], seed_v[pl.ds(192, 64), :]))

    for c in slab_cps[2]:
        c.start()
    for c in slab_cps[0] + slab_cps[1]:
        c.wait()
    for c in slab_cps[3] + slab_cps[4] + xa_cps:
        c.start()
    wrow_s[pl.ds(0, 4), :] = shift_v[...].astype(F32)
    wrow_s[pl.ds(4, 1), :] = ssmd_v[...].astype(F32).reshape(1, DM)
    row0 = lax.broadcasted_iota(jnp.int32, (8, 128), 0) == 0
    RB = 128

    def taps(j):
        lane0 = j * 128
        return ([wrow_s[pl.ds(t, 1), pl.ds(lane0, 128)] for t in range(4)],
                wrow_s[pl.ds(4, 1), pl.ds(lane0, 128)])

    def prep_p(j, r, n):
        kf_s[pl.ds(8 + r, n), :] = k_v[j, pl.ds(r, n), :].astype(F32)

    def prep_q(j, r, w):
        ks = (kf_s[pl.ds(8 + r, RB), :] * w[0] + kf_s[pl.ds(7 + r, RB), :] * w[1]
              + kf_s[pl.ds(6 + r, RB), :] * w[2] + kf_s[pl.ds(5 + r, RB), :] * w[3])
        kv_s[pl.ds(r, RB), :] = ks * v_v[j, pl.ds(r, RB), :].astype(F32)

    def prep_t(j, dd):
        ht = ssmk_v[j].astype(F32).T
        ht_s[pl.ds(8, S_LEN - 8), :] = ht[8:]
        ht_s[pl.ds(0, 8), :] = ht[:8] + jnp.where(row0, dd, np.float32(0.0))

    def pk(re, im):
        return jnp.concatenate([re, im], axis=0).astype(BF16)

    def fwd_nets(src, dst):
        def fwd_a(g, c):
            r = pl.multiple_of(g * 8, 8)
            r2 = pl.multiple_of(g * 16, 16)
            xs = [_SV(src[pl.ds(n2 * 64 + r, 8), :]) for n2 in range(32)]
            orr, oi = _odft(xs)
            for q in range(16):
                dst[2 * q + 1, pl.ds(r2, 16), :] = pk(orr[q].get(), oi[q].get())
            return c

        def fwd_b(g, c):
            r = pl.multiple_of(g * 8, 8)
            r2 = pl.multiple_of(g * 16, 16)
            xs = [_SV(src[pl.ds(n2 * 64 + r, 8), :]) for n2 in range(32)]
            er, ei = _rdft(xs)
            dst[0, pl.ds(r2, 16), :] = pk(er[0].get(), er[16].get())
            for q in range(1, 16):
                dst[2 * q, pl.ds(r2, 16), :] = pk(er[q].get(), ei[q].get())
            return c

        lax.fori_loop(0, 8, fwd_a, 0)
        lax.fori_loop(0, 8, fwd_b, 0)

    def inv_a(br, r):
        sr = [_SV(br[2 * q + 1, pl.ds(r, 8), :]) for q in range(16)]
        si = [_SV(br[2 * q + 1, pl.ds(64 + r, 8), :]) for q in range(16)]
        bb = _odft_T(sr, si)
        for n2 in range(32):
            ta_s[pl.ds(n2 * 64 + r, 8), :] = bb[n2].get()

    def inv_b(br, jy, r):
        sr = [None] * 17
        si = [None] * 17
        sr[0] = _SV(br[0, pl.ds(r, 8), :])
        sr[16] = _SV(br[0, pl.ds(64 + r, 8), :])
        for q in range(1, 16):
            sr[q] = _SV(br[2 * q, pl.ds(r, 8), :])
            si[q] = _SV(br[2 * q, pl.ds(64 + r, 8), :])
        aa = _rdft_T(sr, si)
        for n2 in range(32):
            prev = _SV(ta_s[pl.ds(n2 * 64 + r, 8), :])
            y_v[jy, pl.ds(n2 * 64 + r, 8), :] = (aa[n2] + prev).get()

    def mxu_block(j, bw, br):
        jn = j + 1
        jy = j - 1
        do_prep = j + 1 < NSLAB
        do_inv = j >= 1
        w, dd = taps(min(jn, NSLAB - 1))
        LAG = 3
        X, Y = {}, {}
        for t in range(32 + LAG):
            if do_prep and t % 8 == 0 and t < 32:
                nb = t // 2
                ht_s[pl.ds(nb * 128, 512), :] = ssmk_v[jn, :, pl.ds(nb * 128, 512)].astype(F32).T
            if do_prep and t % 2 == 0 and t < 32:
                prep_p(jn, (t // 2) * RB, RB)
            if do_prep and t % 2 == 1 and t < 32:
                prep_q(jn, (t // 2) * RB, w)
            if do_inv and t % 4 == 0 and t < 32:
                inv_a(br, (t // 4) * 8)
            if do_inv and t % 4 == 2 and t < 32:
                inv_b(br, jy, (t // 4) * 8)
            if t < 32:
                f = pltpu.bitcast(ffw_s[t], BF16)
                X[t] = (_mm(f, akv_s[t]), _mm(f, ah_s[t]))
            if 1 <= t <= 32:
                sl = t - 1
                xk, xh = X.pop(sl)
                kr, ki, hr, hi = xk[:64], xk[64:], xh[:64], xh[64:]
                yr = kr * hr - ki * hi
                yi = kr * hi + ki * hr
                if sl == 0:
                    yr = jnp.concatenate([jnp.where(row0, kr[:8] * hr[:8], yr[:8]), yr[8:]], axis=0)
                    yi = jnp.concatenate([jnp.where(row0, ki[:8] * hi[:8], yi[:8]), yi[8:]], axis=0)
                parts = []
                for jj in range(8):
                    parts.append(yr[8 * jj:8 * jj + 8])
                    parts.append(yi[8 * jj:8 * jj + 8])
                Y[sl] = jnp.concatenate(parts, axis=0).astype(BF16)
            if t >= LAG:
                sl = t - LAG
                bw[sl] = _mm(pltpu.bitcast(fiv_s[sl], BF16), Y.pop(sl))
        if do_prep:
            ht_s[pl.ds(0, 8), :] = ht_s[pl.ds(0, 8), :] + jnp.where(row0, dd, np.float32(0.0))

    w0, dd0 = taps(0)

    def p_body(b, c):
        prep_p(0, pl.multiple_of(b * 256, 256), 256)
        return c

    lax.fori_loop(0, S_LEN // 256, p_body, 0)

    def q_body(b, c):
        prep_q(0, pl.multiple_of(b * RB, RB), w0)
        return c

    lax.fori_loop(0, S_LEN // RB, q_body, 0)
    prep_t(0, dd0)

    for j in range(NSLAB):
        if j == 1:
            for c in w_cps[:W_B0]:
                c.start()
        fwd_nets(kv_s, akv_s)
        fwd_nets(ht_s, ah_s)
        if j == 1:
            for c in slab_cps[2] + slab_cps[3] + slab_cps[4] + xa_cps:
                c.wait()
            for c in w_cps[W_B0:W_B1]:
                c.start()
        if j == 2:
            for c in w_cps[W_B1:] + wo_cps:
                c.start()
        mxu_block(j, (ba_s, bb_s)[j % 2], (ba_s, bb_s)[1 - j % 2])
    jl = NSLAB - 1

    def ia_body(g, c):
        inv_a(ba_s if jl % 2 == 0 else bb_s, pl.multiple_of(g * 8, 8))
        return c

    def ib_body(g, c):
        inv_b(ba_s if jl % 2 == 0 else bb_s, jl, pl.multiple_of(g * 8, 8))
        return c

    lax.fori_loop(0, 8, ia_body, 0)
    lax.fori_loop(0, 8, ib_body, 0)

    for c in w_cps:
        c.wait()

    def relayout_pair(p):
        for m in range(3):
            ia = m * 32 + p
            ib = ia + 16
            for r in range(0, 320, 64):
                a = wbuf[ia, pl.ds(r, 64), :]
                b = wbuf[ib, pl.ds(r, 64), :]
                wbuf[ia, pl.ds(r, 64), :] = (a & np.uint32(0xFFFF)) | (b << 16)
                wbuf[ib, pl.ds(r, 64), :] = (a >> 16) | (b & np.uint32(0xFFFF0000))

    def widx(m, h):
        return m * 32 + (h % 2) * 16 + h // 2

    LAGS_MID = (3, 10, 2)
    LAGS_EDGE = (4, 7, 6)
    cscale = np.float32(DH ** -0.5 * log2e)

    def load_y(idx):
        r0 = pl.multiple_of(idx * SEG, SEG)
        return jnp.concatenate([y_v[jj, pl.ds(r0, SEG), :] for jj in range(NSLAB)], axis=1)

    def wt(m, h):
        return pltpu.bitcast(wbuf[widx(m, h)], BF16)

    def filler(seg):
        rn = pl.multiple_of(seg * SEG, SEG)
        tok1 = _ln(x_v[pl.ds(rn, SEG), :].astype(F32)).astype(BF16)
        for h in range(NF):
            for m in range(3):
                q1_s[h * 3 + m] = _mm(tok1, wt(m, h)).astype(BF16)
        h_s[pl.ds(0, 32), :] = tok1

    def attention(kind):
        r0, r1 = {"first": (0, 48), "mid": (0, 80), "last": (32, 80)}[kind]
        R = r1 - r0
        H = h_s[pl.ds(r0, R), :]
        if kind == "last":
            HQ = h_s[pl.ds(48, 32), :]
            bias = biasl_s[pl.ds(16, 32), :]
        else:
            HQ = H
            bias = bias_s[pl.ds(0, R), :]
        valid = bias > np.float32(-1.0)
        bounds = (0, 8, 16, 24, 32)
        nf = NF if kind == "mid" else 0
        if nf:
            HB = h_s[pl.ds(32, 48), :]
        qkv, P, L, O = {}, {}, {}, {}
        acc = [None] * NSLAB
        zpad = jnp.zeros((128 - R, DH), BF16)

        def do_qkv(h):
            if h < nf:
                qkv[h] = tuple(jnp.concatenate([q1_s[h * 3 + m], _mm(HB, wt(m, h)).astype(BF16)], axis=0)
                               for m in range(3))
            else:
                qkv[h] = tuple(_mm(HQ if m == 0 else H, wt(m, h)).astype(BF16) for m in range(3))

        def do_s(h):
            q, k, v = qkv[h]
            sc = _mm_nt(q, jnp.concatenate([k, zpad], axis=0))
            t = jnp.where(valid, sc * cscale, bias)
            mx = jnp.max(t, axis=-1, keepdims=True)
            e = jnp.exp2(t - mx)
            L[h] = jnp.sum(e, axis=-1, keepdims=True)
            P[h] = e.astype(BF16)

        def do_pv(h):
            v = qkv[h][2]
            o = _mm(P[h], jnp.concatenate([v, zpad], axis=0))
            O[h] = (o * _recip(L[h])).astype(BF16)

        def do_wo(g):
            if kind == "first":
                for ci in range(len(wo_cps)):
                    if WO_SPLIT[ci] == bounds[g]:
                        wo_cps[ci].wait()
                        if ci + 1 == len(wo_cps):
                            xb_cp.start()
            og = jnp.concatenate([O[h] for h in range(bounds[g], bounds[g + 1])], axis=1)
            for n in range(NSLAB):
                wo_n = pltpu.bitcast(wo_v[pl.ds(bounds[g] * 64, (bounds[g + 1] - bounds[g]) * 64),
                                          pl.ds(n * 128, 128)], BF16)
                r = _mm(og, wo_n)
                acc[n] = r if acc[n] is None else acc[n] + r

        NG = len(bounds) - 1
        done_wo = 0
        LAG_S, LAG_PV, LAG_WO = LAGS_MID if kind == "mid" else LAGS_EDGE
        if kind == "first":
            LAG_WO = 2 * NH
        for h in range(NH + LAG_PV + 1):
            if kind == "first" and h % 2 == 0:
                if h == 0:
                    relayout_pair(0)
                if h + 2 < NH:
                    relayout_pair(h // 2 + 1)
            if h < NH:
                do_qkv(h)
            if LAG_S <= h < NH + LAG_S:
                do_s(h - LAG_S)
            if LAG_PV <= h < NH + LAG_PV:
                do_pv(h - LAG_PV)
            while done_wo < NG and bounds[done_wo + 1] - 1 + LAG_PV + LAG_WO <= h:
                do_wo(done_wo)
                done_wo += 1
        while done_wo < NG:
            do_wo(done_wo)
            done_wo += 1
        return acc

    def l2_epilogue(a2, seg):
        x2 = _rb(x1p_s[...] + _rb(a2))
        res = x2 + _rb(_rb(_ln(x2)) * load_y(seg))
        r = pl.multiple_of(seg * SEG, SEG)
        out_v[pl.ds(r, SEG), :] = res.astype(BF16)

    def out_copy(seg):
        r = pl.multiple_of(seg * SEG, SEG)
        return pltpu.make_async_copy(out_v.at[pl.ds(r, SEG), :], out_hbm.at[pl.ds(r, SEG), :], sem_out.at[0])

    def l1_epilogue(a1, seg):
        r1 = pl.multiple_of(seg * SEG, SEG)
        x1 = _rb(x_v[pl.ds(r1, SEG), :].astype(F32) + _rb(a1))
        x1p = _rb(x1 + _rb(_rb(_ln(x1)) * load_y(seg)))
        x1p_s[...] = x1p
        h_s[pl.ds(48, 32), :] = _ln(x1p).astype(BF16)

    mem0 = mem0_v[...]
    h_s[pl.ds(0, 32), :] = _ln(x_v[pl.ds(0, SEG), :].astype(F32)).astype(BF16)
    h_s[pl.ds(32, 16), :] = jnp.concatenate([mem0, mem0], axis=0)
    acc = attention("first")
    filler(1)
    accf = jnp.concatenate(acc, axis=1)
    l1_epilogue(accf[0:32], 0)
    h_s[pl.ds(32, 16), :] = jnp.concatenate([accf[32:40].astype(BF16), mem0], axis=0)

    def mid_step(i):
        acc = attention("mid")
        filler(jnp.minimum(i + 1, NSEG - 1))
        accf = jnp.concatenate(acc, axis=1)
        l2_epilogue(accf[48:80], i - 1)
        l1_epilogue(accf[0:32], i)
        h_s[pl.ds(32, 16), :] = accf[32:48].astype(BF16)
        out_copy(i - 1).start()

    def step(i, carry):
        mid_step(i)

        @pl.when(i == 2)
        def _():
            xb_cp.wait()

        return carry

    lax.fori_loop(1, NSEG, step, 0)

    acc = attention("last")
    accf = jnp.concatenate(acc, axis=1)
    l2_epilogue(accf, NSEG - 1)
    out_copy(NSEG - 1).start()

    def wait_body(i, carry):
        out_copy(i).wait()
        return carry

    lax.fori_loop(0, NSEG, wait_body, 0)


@functools.partial(jax.jit, static_argnames=("A_seg_len",))
def pallas_interleave_layers__memory_aug_recurrent_mem_tr__ssm_conv_h3__prompt_kernel(
    A_x, A_mem0, A_Wq, A_Wk, A_Wv, A_Wo, A_seg_len, B_q, B_k, B_v, B_shift_k, B_ssm_k, B_ssm_D,
):
    del B_q
    assert A_seg_len == SEG
    x = A_x.reshape(S_LEN, DM)
    mem0 = A_mem0.reshape(MEM, DM)
    wq = A_Wq.reshape(DM // 2, 2 * NH, DH)
    wk = A_Wk.reshape(DM // 2, 2 * NH, DH)
    wv = A_Wv.reshape(DM // 2, 2 * NH, DH)
    wo = A_Wo.reshape(NH * DH, DM)
    k = B_k.reshape(S_LEN, DM)
    v = B_v.reshape(S_LEN, DM)
    seed = jnp.asarray(_SEED_TAB)
    any_spec = pl.BlockSpec(memory_space=pl.ANY)
    V = pltpu.VMEM
    DMA = pltpu.SemaphoreType.DMA
    scratch = [
        V((S_LEN, DM), BF16),
        V((MEM, DM), BF16),
        V((96, DM // 2, DH), U32),
        V((NH * DH // 2, DM), U32),
        V((NSLAB, S_LEN, 128), BF16),
        V((NSLAB, S_LEN, 128), BF16),
        V((4, DM), BF16),
        V((NSLAB, 128, S_LEN), BF16),
        V((DM,), BF16),
        V((648, 128), F32),
        V((32, 64, 128), U32),
        V((32, 64, 128), U32),
        V((8, DM), F32),
        V((8 + S_LEN, 128), F32),
        V((S_LEN, 128), F32),
        V((S_LEN, 128), F32),
        V((32, 128, 128), BF16),
        V((32, 128, 128), BF16),
        V((32, 128, 128), F32),
        V((32, 128, 128), F32),
        V((S_LEN, 128), F32),
        V((NSLAB, S_LEN, 128), F32),
        V((S_LEN, DM), BF16),
        V((ROWS, DM), BF16),
        V((3 * NF, SEG, DH), BF16),
        V((SEG, DM), F32),
        V((ROWS, 128), F32),
        V((48, 128), F32),
        DMA((1,)), DMA((NSLAB,)), DMA((2,)), DMA((1,)), DMA((2,)), DMA((1,)),
    ]
    out = pl.pallas_call(
        _kernel,
        out_shape=jax.ShapeDtypeStruct((S_LEN, DM), BF16),
        in_specs=[any_spec] * 12,
        out_specs=any_spec,
        scratch_shapes=scratch,
        compiler_params=pltpu.CompilerParams(vmem_limit_bytes=100 * 1024 * 1024),
    )(x, mem0, wq, wk, wv, wo, k, v, B_shift_k.T, B_ssm_k, B_ssm_D, seed)
    return out.reshape(1, S_LEN, DM)
```
